```python
import jax
import jax.numpy as jnp

def _softmax(x, axis=-1):
    return jax.nn.softmax(x, axis=axis)

def _gelu(x):
    return jax.nn.gelu(x, approximate=True)

def _silu(x):
    return jax.nn.silu(x)

def _sigmoid(x):
    return jax.nn.sigmoid(x)

def _layernorm(x, axis=-1, eps=1e-05):
    m = jnp.mean(x, axis=axis, keepdims=True)
    v = jnp.var(x, axis=axis, keepdims=True)
    return (x - m) / jnp.sqrt(v + eps)

def _scatter_add(tgt, idx, src, axis=0):
    return tgt.at[idx].add(src)

def _segment_sum(src, seg, n):
    return jax.ops.segment_sum(src, seg, n)

class _Rng:

    def __init__(self, key):
        self._k = key

    def _next(self):
        self._k, sub = jax.random.split(self._k)
        return sub

    def normal(self, shape):
        return jax.random.normal(self._next(), shape, dtype=jnp.bfloat16)

    def randint(self, lo, hi, shape):
        return jax.random.randint(self._next(), shape, lo, hi, dtype=jnp.int32)

    def uniform(self, shape, lo=0.0, hi=1.0):
        return jax.random.uniform(self._next(), shape, jnp.bfloat16, lo, hi)

    def permutation(self, n):
        return jax.random.permutation(self._next(), n)
kernel_name = 'interleave_layers__memory_aug_recurrent_mem_tr__moe_arch_mod__prompt'

def setup_inputs():
    _rng = _Rng(jax.random.key(int.from_bytes(__import__("os").urandom(4), "little")))
    _w = lambda a: (lambda t: t.astype(jnp.bfloat16) if jnp.issubdtype(t.dtype, jnp.floating) else t)(jnp.asarray(a))

    def _A_setup():
        B, S, Dm = (1, 2048, 512)
        H, Dh = (32, 128)
        M, seg = (8, 32)
        seg = min(seg, S)
        S = S // seg * seg
        return {'x': _w((lambda *s: _rng.normal(s) * 0.05)(B, S, Dm)), 'mem0': _w((lambda *s: _rng.normal(s) * 0.05)(B, M, Dm)), 'Wq': _w((lambda *s: _rng.normal(s) * 0.05)(Dm, H, Dh) * Dm ** (-0.5)), 'Wk': _w((lambda *s: _rng.normal(s) * 0.05)(Dm, H, Dh) * Dm ** (-0.5)), 'Wv': _w((lambda *s: _rng.normal(s) * 0.05)(Dm, H, Dh) * Dm ** (-0.5)), 'Wo': _w((lambda *s: _rng.normal(s) * 0.05)(H, Dh, Dm) * (H * Dh) ** (-0.5)), 'seg_len': seg}
    _A_in = _A_setup()

    def _B_setup():
        B, S, D, F, C = (1, 2048, 512, 1792, 1)
        return {'x': _w((lambda *s: _rng.normal(s) * 0.05)(B, S, D)), 'w_r': _w((lambda *s: _rng.normal(s) * 0.05)(D)), 'w_gate': _w((lambda *s: _rng.normal(s) * 0.05)(D, F)), 'w_up': _w((lambda *s: _rng.normal(s) * 0.05)(D, F)), 'w_down': _w((lambda *s: _rng.normal(s) * 0.05)(F, D))}
    _B_in = _B_setup()
    return {'A_x': _A_in['x'], 'A_mem0': _A_in['mem0'], 'A_Wq': _A_in['Wq'], 'A_Wk': _A_in['Wk'], 'A_Wv': _A_in['Wv'], 'A_Wo': _A_in['Wo'], 'A_seg_len': _A_in['seg_len'], 'B_x': _B_in['x'], 'B_w_r': _B_in['w_r'], 'B_w_gate': _B_in['w_gate'], 'B_w_up': _B_in['w_up'], 'B_w_down': _B_in['w_down']}

def reference(A_x, A_mem0, A_Wq, A_Wk, A_Wv, A_Wo, A_seg_len, B_x, B_w_r, B_w_gate, B_w_up, B_w_down):

    def _A_ref(x, mem0, Wq, Wk, Wv, Wo, seg_len):
        B, S, Dm = x.shape
        H, Dh = (Wq.shape[1], Wq.shape[2])
        M = mem0.shape[1]
        scale = Dh ** (-0.5)
        n_seg = S // seg_len
        L = M + seg_len
        idx = jnp.arange(L)
        mask = (idx[:, None] < M) | (idx[:, None] >= idx[None, :])
        mem = mem0
        outs = []
        for s in range(n_seg):
            xs = x[:, s * seg_len:(s + 1) * seg_len, :].copy()
            h = jnp.concatenate([mem, xs], axis=1)
            q = jnp.einsum('btd,dhe->bhte', h, Wq)
            k = jnp.einsum('btd,dhe->bhte', h, Wk)
            v = jnp.einsum('btd,dhe->bhte', h, Wv)
            scores = jnp.einsum('bhqe,bhke->bhqk', q, k) * scale
            scores = jnp.where(mask[None, None], scores, -1000000000.0)
            p = _softmax(scores, axis=-1)
            o = jnp.einsum('bhqk,bhke->bhqe', p, v)
            o = jnp.einsum('bhte,hed->btd', o, Wo)
            mem = o[:, :M, :].copy()
            outs.append(o[:, M:, :])
        return jnp.concatenate(outs, axis=1)

    def _B_ref(x, w_r, w_gate, w_up, w_down):
        B, S, D = x.shape
        C = 1
        r = x @ w_r
        idx = jnp.argsort(-r, axis=-1)[:, :C]
        idx_e = jnp.repeat(idx.reshape(B, C, 1), D, axis=2)
        x_sel = jnp.take_along_axis(x, idx_e, axis=1)
        g = _silu(x_sel @ w_gate)
        u = x_sel @ w_up
        y = g * u @ w_down
        r_sel = _sigmoid(jnp.take_along_axis(r, idx, axis=1))
        y = y * r_sel.reshape(B, C, 1)
        b_off = (jnp.arange(B) * S).reshape(B, 1)
        flat_idx = (idx + b_off).reshape(B * C)
        zero = (x * 0.0).reshape(B * S, D)
        upd = _scatter_add(zero, flat_idx, y.reshape(B * C, D), axis=0)
        return x + upd.reshape(B, S, D)
    x = A_x
    x = x + _A_ref(_layernorm(x, axis=-1), A_mem0, A_Wq, A_Wk, A_Wv, A_Wo, A_seg_len)
    x = x + _B_ref(_layernorm(x, axis=-1), B_w_r, B_w_gate, B_w_up, B_w_down)
    x = x + _A_ref(_layernorm(x, axis=-1), A_mem0, A_Wq, A_Wk, A_Wv, A_Wo, A_seg_len)
    x = x + _B_ref(_layernorm(x, axis=-1), B_w_r, B_w_gate, B_w_up, B_w_down)
    return x
```

```python
import functools

import jax
import jax.numpy as jnp
import numpy as np
from jax import lax
import jax.experimental.pallas as pl
import jax.experimental.pallas.tpu as pltpu

_F32 = jnp.float32
_BF16 = jnp.bfloat16
_LANES = 128
_NN = (((1,), (0,)), ((), ()))
_NT = (((1,), (1,)), ((), ()))


def _dot(a, b, dims=_NN):
    return lax.dot_general(a, b, dims, preferred_element_type=_F32)


def _rnd(a):
    return a.astype(_BF16).astype(_F32)


def _layernorm(x):
    inv_n = np.float32(1.0 / x.shape[-1])
    mean = jnp.sum(x, axis=-1, keepdims=True) * inv_n
    cen = x - mean
    var = jnp.sum(cen * cen, axis=-1, keepdims=True) * inv_n
    eps = np.float32(np.asarray(1e-05).astype(_BF16))
    den = _rnd(jnp.sqrt(_rnd(_rnd(var) + eps)))
    return _rnd(_rnd(x - _rnd(mean)) * (1.0 / den))


def _sigmoid(x):
    return 1.0 / (1.0 + jnp.exp(-x))


def _kernel(
    x_hbm, mem0_ref, wq_hbm, wk_hbm, wv_hbm, wo_hbm, wr_ref, wg_hbm, wu_hbm, wd_hbm,
    out_hbm,
    wraw, wqkv, wo, wg, wu, wd, xres, zbuf, x1buf, z1buf, obuf, sems,
    *, seg, n_heads, n_chunks,
):
    S, D = x_hbm.shape
    M = mem0_ref.shape[0]
    L = M + seg
    n_seg = S // seg
    n_col = D // _LANES
    scale = _LANES ** -0.5

    rows_per_chunk = D * n_heads // n_chunks
    x_copy = pltpu.make_async_copy(x_hbm, xres.at[pl.ds(0, S)], sems.at[0])
    w_copies = [
        pltpu.make_async_copy(
            w.at[pl.ds(c * rows_per_chunk, rows_per_chunk)],
            wraw.at[i * n_chunks + c],
            sems.at[8 + i * n_chunks + c])
        for i, w in enumerate((wq_hbm, wk_hbm, wv_hbm)) for c in range(n_chunks)
    ]
    wo_copies = [
        pltpu.make_async_copy(wo_hbm.at[:, pl.ds(j * _LANES, _LANES)], wo.at[j], sems.at[1])
        for j in range(n_col)
    ]
    ffn_copies = [
        pltpu.make_async_copy(src, dst, sems.at[2 + i])
        for i, (src, dst) in enumerate(((wg_hbm, wg), (wu_hbm, wu), (wd_hbm, wd)))
    ]
    x_copy.start()
    for cp in w_copies + wo_copies + ffn_copies:
        cp.start()

    xres[pl.ds(S, seg), :] = jnp.zeros((seg, D), _BF16)
    obuf[...] = jnp.zeros(obuf.shape, _F32)

    x_copy.wait()

    def first_norm(i, _):
        rows = pl.ds(pl.multiple_of(i * 128, 128), 128)
        zbuf[rows, :] = _layernorm(xres[rows, :].astype(_F32))
    lax.fori_loop(0, S // 128, first_norm, None)

    d_per_chunk = D // n_chunks
    pairs = n_heads // 2
    for n, cp in enumerate(w_copies):
        cp.wait()
        i, c = divmod(n, n_chunks)

        def split_heads(b, _, n=n, i=i, c=c):
            src = pl.ds(pl.multiple_of(b * (32 * n_heads), 32 * n_heads), 32 * n_heads)
            words = wraw.at[n, src].bitcast(jnp.uint32)
            rows = pl.ds(pl.multiple_of(c * d_per_chunk + b * 32, 32), 32)
            for p in range(pairs):
                w = words[pl.ds(p, 32, stride=pairs), :]
                even = pltpu.bitcast(w << 16, _F32).astype(_BF16)
                odd = pltpu.bitcast(w & np.uint32(0xFFFF0000), _F32).astype(_BF16)
                wqkv[i * n_heads + 2 * p, rows, :] = even
                wqkv[i * n_heads + 2 * p + 1, rows, :] = odd
        lax.fori_loop(0, d_per_chunk // 32, split_heads, None)

    for cp in wo_copies:
        cp.wait()

    qi = lax.broadcasted_iota(jnp.int32, (L, L), 0)
    ki = lax.broadcasted_iota(jnp.int32, (L, L), 1)
    visible = (qi < M) | (qi >= ki)
    w_r = wr_ref[...].astype(_F32)

    def post(s, best, best_idx):
        slot = jnp.where(s < 0, n_seg, s)
        rows = pl.ds(pl.multiple_of(slot * seg, seg), seg)
        x1 = _rnd(xres[rows, :].astype(_F32) + _rnd(obuf[...]))
        z1 = _layernorm(x1)
        x2 = (x1 + z1).astype(_BF16)
        x1buf[rows, :] = x1
        z1buf[rows, :] = z1
        xres[rows, :] = x2
        zbuf[rows, :] = _layernorm(x2.astype(_F32))
        r = _rnd(jnp.sum(z1 * w_r, axis=-1, keepdims=True))
        idx = s * seg + lax.broadcasted_iota(jnp.int32, (seg, 1), 0)
        better = (r > best) & (idx >= 0)
        return jnp.where(better, r, best), jnp.where(better, idx, best_idx)

    def step(s, carry):
        mem, best, best_idx = carry
        z = zbuf[pl.ds(pl.multiple_of(s * seg, seg), seg), :]
        h = jnp.concatenate([mem, z], axis=0)
        best, best_idx = post(s - 1, best, best_idx)
        heads = []
        for hd in range(n_heads):
            q = _dot(h, wqkv[hd])
            k = _dot(h, wqkv[n_heads + hd])
            v = _dot(h, wqkv[2 * n_heads + hd])
            sc = jnp.where(visible, _dot(q, k, _NT) * scale, -1000000000.0)
            e = jnp.exp(sc - jnp.max(sc, axis=-1, keepdims=True))
            den = jnp.sum(e, axis=-1, keepdims=True)
            heads.append(_dot(e, v) * (1.0 / den))
        o = jnp.concatenate(heads, axis=1)
        out = jnp.concatenate([_dot(o, wo[j]) for j in range(n_col)], axis=1)
        obuf[...] = out[M:]
        return out[:M], best, best_idx

    def layer(l, _):
        init = (
            mem0_ref[...].astype(_F32),
            jnp.full((seg, 1), -np.inf, _F32),
            lax.broadcasted_iota(jnp.int32, (seg, 1), 0),
        )
        _, best, best_idx = lax.fori_loop(0, n_seg, step, init)
        best, best_idx = post(n_seg - 1, best, best_idx)

        top = jnp.max(best, axis=0, keepdims=True)
        idx = jnp.min(jnp.where(best == top, best_idx, S - 1))

        @pl.when(l == 0)
        def _():
            for cp in ffn_copies:
                cp.wait()

        rows = pl.ds(pl.multiple_of((idx // 16) * 16, 16), 16)
        z1 = z1buf[rows, :]
        gate = _rnd(_dot(z1, wg[...]))
        g = _rnd(gate * _rnd(_sigmoid(gate)))
        u = _rnd(_dot(z1, wu[...]))
        y = _rnd(_dot(g * u, wd[...]))
        y = _rnd(y * _rnd(_sigmoid(top)))
        picked = lax.broadcasted_iota(jnp.int32, (16, D), 0) == idx % 16
        x2 = (x1buf[rows, :] + jnp.where(picked, _rnd(z1 + y), z1)).astype(_BF16)
        xres[rows, :] = x2
        zbuf[rows, :] = _layernorm(x2.astype(_F32))

    lax.fori_loop(0, 2, layer, None)

    out_copy = pltpu.make_async_copy(xres.at[pl.ds(0, S)], out_hbm, sems.at[5])
    out_copy.start()
    out_copy.wait()


@functools.partial(jax.jit, static_argnames=("A_seg_len",))
def pallas_interleave_layers__memory_aug_recurrent_mem_tr__moe_arch_mod__prompt_kernel(
    A_x: jax.Array,
    A_mem0: jax.Array,
    A_Wq: jax.Array,
    A_Wk: jax.Array,
    A_Wv: jax.Array,
    A_Wo: jax.Array,
    A_seg_len: int,
    B_x: jax.Array,
    B_w_r: jax.Array,
    B_w_gate: jax.Array,
    B_w_up: jax.Array,
    B_w_down: jax.Array,
):
    del B_x
    B, S, D = A_x.shape
    M = A_mem0.shape[1]
    H, Dh = A_Wq.shape[1:]
    F = B_w_gate.shape[1]
    seg = int(A_seg_len)
    assert B == 1 and Dh == _LANES and S % seg == 0 and seg % 16 == 0 and M % 8 == 0
    n_chunks = 4

    hbm = pl.BlockSpec(memory_space=pl.ANY)
    vmem = pl.BlockSpec(memory_space=pltpu.VMEM)
    out = pl.pallas_call(
        functools.partial(_kernel, seg=seg, n_heads=H, n_chunks=n_chunks),
        out_shape=jax.ShapeDtypeStruct((S, D), A_x.dtype),
        in_specs=[hbm, vmem, hbm, hbm, hbm, hbm, vmem, hbm, hbm, hbm],
        out_specs=hbm,
        scratch_shapes=[
            pltpu.VMEM((3 * n_chunks, D * H // n_chunks, Dh), _BF16),
            pltpu.VMEM((3 * H, D, Dh), _BF16),
            pltpu.VMEM((D // _LANES, H * Dh, _LANES), _BF16),
            pltpu.VMEM((D, F), _BF16),
            pltpu.VMEM((D, F), _BF16),
            pltpu.VMEM((F, D), _BF16),
            pltpu.VMEM((S + seg, D), _BF16),
            pltpu.VMEM((S + seg, D), _F32),
            pltpu.VMEM((S + seg, D), _F32),
            pltpu.VMEM((S + seg, D), _F32),
            pltpu.VMEM((seg, D), _F32),
            pltpu.SemaphoreType.DMA((8 + 3 * n_chunks,)),
        ],
        compiler_params=pltpu.CompilerParams(vmem_limit_bytes=100 * 1024 * 1024),
        name="rmt_mod",
    )(
        A_x.reshape(S, D),
        A_mem0.reshape(M, D),
        A_Wq.reshape(D * H, Dh),
        A_Wk.reshape(D * H, Dh),
        A_Wv.reshape(D * H, Dh),
        A_Wo.reshape(H * Dh, D),
        B_w_r.reshape(1, D),
        B_w_gate,
        B_w_up,
        B_w_down,
    )
    return out.reshape(B, S, D)
```

```python
import functools

import jax
import jax.numpy as jnp
import numpy as np
from jax import lax
import jax.experimental.pallas as pl
import jax.experimental.pallas.tpu as pltpu

_F32 = jnp.float32
_BF16 = jnp.bfloat16
_LANES = 128
_NN = (((1,), (0,)), ((), ()))
_NT = (((1,), (1,)), ((), ()))


def _dot(a, b, dims=_NN):
    return lax.dot_general(a, b, dims, preferred_element_type=_F32)


def _rnd(a):
    return a.astype(_BF16).astype(_F32)


def _layernorm(x):
    inv_n = np.float32(1.0 / x.shape[-1])
    mean = jnp.sum(x, axis=-1, keepdims=True) * inv_n
    cen = x - mean
    var = jnp.sum(cen * cen, axis=-1, keepdims=True) * inv_n
    eps = np.float32(np.asarray(1e-05).astype(_BF16))
    den = _rnd(jnp.sqrt(_rnd(_rnd(var) + eps)))
    return _rnd(_rnd(x - _rnd(mean)) * (1.0 / den))


def _sigmoid(x):
    return 1.0 / (1.0 + jnp.exp(-x))


def _kernel(
    x_hbm, mem0_ref, wq_hbm, wk_hbm, wv_hbm, wo_hbm, wr_ref, wg_hbm, wu_hbm, wd_hbm,
    out_hbm,
    wraw, wqkv, wo, wg, wu, wd, xres, zbuf, x1buf, z1buf, obuf, sems,
    *, seg, n_heads, n_chunks,
):
    S, D = x_hbm.shape
    M = mem0_ref.shape[0]
    L = M + seg
    n_seg = S // seg
    n_col = D // _LANES
    scale = _LANES ** -0.5

    rows_per_chunk = D * n_heads // n_chunks
    x_copy = pltpu.make_async_copy(x_hbm, xres.at[pl.ds(0, S)], sems.at[0])
    w_copies = [
        pltpu.make_async_copy(
            w.at[pl.ds(c * rows_per_chunk, rows_per_chunk)],
            wraw.at[i * n_chunks + c],
            sems.at[8 + i * n_chunks + c])
        for i, w in enumerate((wq_hbm, wk_hbm, wv_hbm)) for c in range(n_chunks)
    ]
    wo_copies = [
        pltpu.make_async_copy(wo_hbm.at[:, pl.ds(j * _LANES, _LANES)], wo.at[j], sems.at[1])
        for j in range(n_col)
    ]
    ffn_copies = [
        pltpu.make_async_copy(src, dst, sems.at[2 + i])
        for i, (src, dst) in enumerate(((wg_hbm, wg), (wu_hbm, wu), (wd_hbm, wd)))
    ]
    x_copy.start()
    for cp in w_copies + wo_copies + ffn_copies:
        cp.start()

    xres[pl.ds(S, seg), :] = jnp.zeros((seg, D), _BF16)
    obuf[...] = jnp.zeros(obuf.shape, _F32)

    x_copy.wait()

    def first_norm(i, _):
        rows = pl.ds(pl.multiple_of(i * 128, 128), 128)
        zbuf[rows, :] = _layernorm(xres[rows, :].astype(_F32))
    lax.fori_loop(0, S // 128, first_norm, None)

    d_per_chunk = D // n_chunks
    pairs = n_heads // 2
    for n, cp in enumerate(w_copies):
        cp.wait()
        i, c = divmod(n, n_chunks)

        def split_heads(b, _, n=n, i=i, c=c):
            src = pl.ds(pl.multiple_of(b * (32 * n_heads), 32 * n_heads), 32 * n_heads)
            words = wraw.at[n, src].bitcast(jnp.uint32)
            rows = pl.ds(pl.multiple_of((c * d_per_chunk + b * 32) // 2, 16), 16)
            for p in range(pairs):
                w = words[pl.ds(p, 32, stride=pairs), :]
                even = pltpu.bitcast(w << 16, _F32).astype(_BF16)
                odd = pltpu.bitcast(w & np.uint32(0xFFFF0000), _F32).astype(_BF16)
                wqkv[i * n_heads + 2 * p, rows, :] = pltpu.bitcast(even, jnp.uint32)
                wqkv[i * n_heads + 2 * p + 1, rows, :] = pltpu.bitcast(odd, jnp.uint32)
        lax.fori_loop(0, d_per_chunk // 32, split_heads, None)

    for cp in wo_copies:
        cp.wait()

    qi = lax.broadcasted_iota(jnp.int32, (L, L), 0)
    ki = lax.broadcasted_iota(jnp.int32, (L, L), 1)
    visible = (qi < M) | (qi >= ki)
    w_r = wr_ref[...].astype(_F32)

    def post(s, best, best_idx):
        slot = jnp.where(s < 0, n_seg, s)
        rows = pl.ds(pl.multiple_of(slot * seg, seg), seg)
        x1 = _rnd(xres[rows, :].astype(_F32) + _rnd(obuf[...]))
        z1 = _layernorm(x1)
        x2 = (x1 + z1).astype(_BF16)
        x1buf[rows, :] = x1
        z1buf[rows, :] = z1
        xres[rows, :] = x2
        zbuf[rows, :] = _layernorm(x2.astype(_F32))
        r = _rnd(jnp.sum(z1 * w_r, axis=-1, keepdims=True))
        idx = s * seg + lax.broadcasted_iota(jnp.int32, (seg, 1), 0)
        better = (r > best) & (idx >= 0)
        return jnp.where(better, r, best), jnp.where(better, idx, best_idx)

    def step(s, carry):
        mem, best, best_idx = carry
        z = zbuf[pl.ds(pl.multiple_of(s * seg, seg), seg), :]
        h = jnp.concatenate([mem, z], axis=0)
        best, best_idx = post(s - 1, best, best_idx)
        G = 4
        n_grp = n_heads // G
        W = lambda i: pltpu.bitcast(wqkv[i], _BF16)
        WO = lambda j, g: wo[j, pl.ds(g * G * _LANES, G * _LANES), :]
        heads = [None] * n_grp
        pend = None

        def finish(pend):
            return jnp.concatenate([_dot(e, v) * inv for e, v, inv in pend], axis=1)

        for g in range(n_grp):
            hs = range(g * G, (g + 1) * G)
            ks = [_dot(h, W(n_heads + hd)) for hd in hs]
            qs = [_dot(h, W(hd)) for hd in hs]
            if pend is not None:
                heads[g - 1] = finish(pend)
            vs = [_dot(h, W(2 * n_heads + hd)) for hd in hs]
            scs = [_dot(q, k, _NT) for q, k in zip(qs, ks)]
            pend = []
            for sc, v in zip(scs, vs):
                sc = jnp.where(visible, sc * scale, -1000000000.0)
                e = jnp.exp(sc - jnp.max(sc, axis=-1, keepdims=True))
                den = jnp.sum(e, axis=-1, keepdims=True)
                pend.append((e, v, 1.0 / den))
        outs = [None] * n_col
        for g in range(n_grp):
            if g == 2:
                heads[n_grp - 1] = finish(pend)
            for j in range(n_col):
                t = _dot(heads[g], WO(j, g))
                outs[j] = t if outs[j] is None else outs[j] + t
        out = jnp.concatenate(outs, axis=1)
        obuf[...] = out[M:]
        return out[:M], best, best_idx

    def layer(l, _):
        init = (
            mem0_ref[...].astype(_F32),
            jnp.full((seg, 1), -np.inf, _F32),
            lax.broadcasted_iota(jnp.int32, (seg, 1), 0),
        )
        _, best, best_idx = lax.fori_loop(0, n_seg, step, init)
        best, best_idx = post(n_seg - 1, best, best_idx)

        top = jnp.max(best, axis=0, keepdims=True)
        idx = jnp.min(jnp.where(best == top, best_idx, S - 1))

        @pl.when(l == 0)
        def _():
            for cp in ffn_copies:
                cp.wait()

        rows = pl.ds(pl.multiple_of((idx // 16) * 16, 16), 16)
        z1 = z1buf[rows, :]
        gate = _rnd(_dot(z1, wg[...]))
        g = _rnd(gate * _rnd(_sigmoid(gate)))
        u = _rnd(_dot(z1, wu[...]))
        y = _rnd(_dot(g * u, wd[...]))
        y = _rnd(y * _rnd(_sigmoid(top)))
        picked = lax.broadcasted_iota(jnp.int32, (16, D), 0) == idx % 16
        x2 = (x1buf[rows, :] + jnp.where(picked, _rnd(z1 + y), z1)).astype(_BF16)
        xres[rows, :] = x2
        zbuf[rows, :] = _layernorm(x2.astype(_F32))

    lax.fori_loop(0, 2, layer, None)

    out_copy = pltpu.make_async_copy(xres.at[pl.ds(0, S)], out_hbm, sems.at[5])
    out_copy.start()
    out_copy.wait()


@functools.partial(jax.jit, static_argnames=("A_seg_len",))
def pallas_interleave_layers__memory_aug_recurrent_mem_tr__moe_arch_mod__prompt_kernel(
    A_x: jax.Array,
    A_mem0: jax.Array,
    A_Wq: jax.Array,
    A_Wk: jax.Array,
    A_Wv: jax.Array,
    A_Wo: jax.Array,
    A_seg_len: int,
    B_x: jax.Array,
    B_w_r: jax.Array,
    B_w_gate: jax.Array,
    B_w_up: jax.Array,
    B_w_down: jax.Array,
):
    del B_x
    B, S, D = A_x.shape
    M = A_mem0.shape[1]
    H, Dh = A_Wq.shape[1:]
    F = B_w_gate.shape[1]
    seg = int(A_seg_len)
    assert B == 1 and Dh == _LANES and S % seg == 0 and seg % 16 == 0 and M % 8 == 0
    n_chunks = 4

    hbm = pl.BlockSpec(memory_space=pl.ANY)
    vmem = pl.BlockSpec(memory_space=pltpu.VMEM)
    out = pl.pallas_call(
        functools.partial(_kernel, seg=seg, n_heads=H, n_chunks=n_chunks),
        out_shape=jax.ShapeDtypeStruct((S, D), A_x.dtype),
        in_specs=[hbm, vmem, hbm, hbm, hbm, hbm, vmem, hbm, hbm, hbm],
        out_specs=hbm,
        scratch_shapes=[
            pltpu.VMEM((3 * n_chunks, D * H // n_chunks, Dh), _BF16),
            pltpu.VMEM((3 * H, D // 2, Dh), jnp.uint32),
            pltpu.VMEM((D // _LANES, H * Dh, _LANES), _BF16),
            pltpu.VMEM((D, F), _BF16),
            pltpu.VMEM((D, F), _BF16),
            pltpu.VMEM((F, D), _BF16),
            pltpu.VMEM((S + seg, D), _BF16),
            pltpu.VMEM((S + seg, D), _F32),
            pltpu.VMEM((S + seg, D), _F32),
            pltpu.VMEM((S + seg, D), _F32),
            pltpu.VMEM((seg, D), _F32),
            pltpu.SemaphoreType.DMA((8 + 3 * n_chunks,)),
        ],
        compiler_params=pltpu.CompilerParams(vmem_limit_bytes=100 * 1024 * 1024),
        name="rmt_mod",
    )(
        A_x.reshape(S, D),
        A_mem0.reshape(M, D),
        A_Wq.reshape(D * H, Dh),
        A_Wk.reshape(D * H, Dh),
        A_Wv.reshape(D * H, Dh),
        A_Wo.reshape(H * Dh, D),
        B_w_r.reshape(1, D),
        B_w_gate,
        B_w_up,
        B_w_down,
    )
    return out.reshape(B, S, D)
```

```python
import functools

import jax
import jax.numpy as jnp
import numpy as np
from jax import lax
import jax.experimental.pallas as pl
import jax.experimental.pallas.tpu as pltpu

CFG = dict(unroll=8, ksplit=1, wo_order="g", pv_last_at=2, G=4, post_pos=0, nshift=4, pack="", n_early=40, zb=1, flags=None, carry_z=0)
CFG.update(unroll=4)

_F32 = jnp.float32
_BF16 = jnp.bfloat16
_U32 = jnp.uint32
_LANES = 128
_EARLY = 8
_NN = (((1,), (0,)), ((), ()))
_NT = (((1,), (1,)), ((), ()))
_K, _Q, _V = range(3)


def _dot(a, b, dims=_NN):
    return lax.dot_general(a, b, dims, preferred_element_type=_F32)


def _rnd(a):
    return a.astype(_BF16).astype(_F32)


def _layernorm_stages(x):
    inv_n = np.float32(1.0 / x.shape[-1])
    mean = jnp.sum(x, axis=-1, keepdims=True) * inv_n
    yield
    cen = x - mean
    var = jnp.sum(cen * cen, axis=-1, keepdims=True) * inv_n
    yield
    eps = np.float32(np.asarray(1e-05).astype(_BF16))
    den = _rnd(jnp.sqrt(_rnd(_rnd(var) + eps)))
    return _rnd(_rnd(x - _rnd(mean)) * (1.0 / den))


class _Staged:
    def __init__(self, stages):
        self._stages, self._result = stages, []

    def advance(self):
        if not self._result:
            try:
                next(self._stages)
            except StopIteration as done:
                self._result.append(done.value)

    def finish(self):
        while not self._result:
            self.advance()
        return self._result[0]


def _layernorm(x):
    return _Staged(_layernorm_stages(x)).finish()


def _sigmoid(x):
    return 1.0 / (1.0 + jnp.exp(-x))


def _kernel(
    x_hbm, mem0_ref, wq_hbm, wk_hbm, wv_hbm, wo_hbm, wr_ref, wg_hbm, wu_hbm, wd_hbm,
    out_hbm,
    wraw, wkqv, wo, wg, wu, wd, xres, zbuf, x1buf, obuf, zearly, early, fixed,
    w_sems, sems,
    *, n_heads,
):
    n_seg, seg, D = x_hbm.shape
    M = mem0_ref.shape[0]
    L = M + seg
    n_col = D // _LANES
    half = _LANES // 2
    scale = _LANES ** -0.5
    unroll = CFG["unroll"]
    n_early = CFG["n_early"]

    def x_copy(first, count, row, rows, sem):
        where = (pl.ds(first, count), pl.ds(row, rows))
        return pltpu.make_async_copy(x_hbm.at[where], xres.at[where], sems.at[sem])

    x_early_copy = x_copy(0, n_early, 0, _EARLY, 0)
    x_late_copy = x_copy(0, n_early, _EARLY, seg - _EARLY, 6)
    x_next_copy = x_copy(n_early, 1, 0, seg, 7)
    x_rest_copy = x_copy(n_early + 1, n_seg - n_early - 1, 0, seg, 8)
    wo_copies = [
        pltpu.make_async_copy(
            wo_hbm.at[:, pl.ds(j * _LANES, _LANES)], wo.at[j].bitcast(_BF16), sems.at[1])
        for j in range(n_col)
    ]
    ffn_copies = [
        pltpu.make_async_copy(src, dst.bitcast(_BF16), sems.at[2 + i])
        for i, (src, dst) in enumerate(((wg_hbm, wg), (wu_hbm, wu), (wd_hbm, wd)))
    ]
    x_early_copy.start()
    for i, w in enumerate((wk_hbm, wq_hbm, wv_hbm)):
        for c in range(n_col):
            n = i * n_col + c
            pltpu.make_async_copy(
                w.at[pl.ds(c * _LANES * n_heads, _LANES * n_heads)], wraw.at[n], w_sems.at[n]
            ).start()
    for cp in [x_late_copy, x_next_copy] + wo_copies + [x_rest_copy] + ffn_copies:
        cp.start()

    xres[n_seg] = jnp.zeros((seg, D), _BF16)
    obuf[...] = jnp.zeros(obuf.shape, _F32)

    x_early_copy.wait()
    x = jnp.concatenate(
        [xres[t, pl.ds(0, _EARLY), :].astype(_F32) for t in range(n_early)], axis=0)
    z = _layernorm(x).astype(zearly.dtype)
    for c in range(n_col):
        zearly[c] = z[:, c * _LANES:(c + 1) * _LANES]

    def unpack_and_project(n, _):
        pltpu.make_async_copy(wraw.at[n], wraw.at[n], w_sems.at[n]).wait()
        which, c = n // n_col, n % n_col
        words = wraw.at[n].bitcast(_U32)
        rows = pl.ds(pl.multiple_of(c * half, half), half)
        z = zearly[c]
        w_out, acc = wkqv.at[which], early.at[which]
        for p in range(n_heads // 2):
            w = words[pl.ds(p, _LANES, stride=n_heads // 2), :]
            pair = (w << 16, w & np.uint32(0xFFFF0000))
            for hd, bits in enumerate(pair, 2 * p):
                w_head = pltpu.bitcast(bits, _F32).astype(_BF16)
                w_out[hd, rows, :] = pltpu.bitcast(w_head, _U32)
                acc[hd] = _dot(z, w_head) + jnp.where(c > 0, acc[hd], 0.0)
    lax.fori_loop(0, 3 * n_col, unpack_and_project, None)

    x_late_copy.wait()
    x_next_copy.wait()
    zbuf[0] = _layernorm(xres[0].astype(_F32))
    for cp in wo_copies:
        cp.wait()

    qi = lax.broadcasted_iota(jnp.int32, (L, L), 0)
    ki = lax.broadcasted_iota(jnp.int32, (L, L), 1)
    visible = (qi >= seg) | (ki >= seg) | (qi >= ki)
    w_r = wr_ref[...].astype(_F32)

    def post(s, best, best_idx):
        slot = jnp.where(s < 0, n_seg, s)
        x1 = _rnd(xres[slot].astype(_F32) + _rnd(obuf[...]))
        x1buf[slot] = x1
        z1 = yield from _layernorm_stages(x1)
        yield
        r = _rnd(jnp.sum(z1 * w_r, axis=-1, keepdims=True))
        idx = s * seg + lax.broadcasted_iota(jnp.int32, (seg, 1), 0)
        better = (r > best) & (idx >= 0)
        xres[slot] = (x1 + z1).astype(_BF16)
        return jnp.where(better, r, best), jnp.where(better, idx, best_idx)

    def pre(s):
        zbuf[s] = yield from _layernorm_stages(xres[s].astype(_F32))

    G = CFG["G"]
    n_grp = n_heads // G
    log2e = float(np.log2(np.e))

    def step(s, carry, first, ahead):
        mem, best, best_idx = carry
        heads = [None] * n_grp
        pend = None
        previous = _Staged(post(s - 1, best, best_idx))
        following = _Staged(pre(s + 1))
        if ahead:
            h = jnp.concatenate([zbuf[s, pl.ds(_EARLY, seg - _EARLY), :], mem], axis=0)
            early_rows = pl.ds(pl.multiple_of(s * _EARLY, _EARLY), _EARLY)
        else:
            h = jnp.concatenate([zbuf[s], mem], axis=0)

        def project(which, hds, by_column=False):
            if by_column:
                res = [None] * len(hds)
                for c in range(n_col):
                    for n, hd in enumerate(hds):
                        w = pltpu.bitcast(wkqv[which, hd, pl.ds(c * half, half), :], _BF16)
                        t = _dot(h[:, c * _LANES:(c + 1) * _LANES], w)
                        res[n] = t if c == 0 else res[n] + t
            else:
                res = [_dot(h, pltpu.bitcast(wkqv[which, hd], _BF16)) for hd in hds]
            if ahead:
                res = [jnp.concatenate([early[which, hd, early_rows, :], r], axis=0)
                       for hd, r in zip(hds, res)]
            if "kqv"[which] in CFG["pack"]:
                res = [r.astype(_BF16) for r in res]
            return res

        def attend(pend):
            o = jnp.concatenate([_dot(e, v) * inv for e, v, inv in pend], axis=1)
            return jnp.concatenate([o[seg:], o[:seg]], axis=0)

        for g in range(n_grp):
            if g >= CFG["post_pos"]:
                previous.advance()
            if g >= CFG["nshift"]:
                following.advance()
            hds = range(g * G, (g + 1) * G)
            ks = project(_K, hds, by_column=g == 0 and CFG["ksplit"] and not first)
            qs = project(_Q, hds)
            if pend is not None:
                heads[g - 1] = attend(pend)
            vs = project(_V, hds)
            scs = [_dot(q, k, _NT) for q, k in zip(qs, ks)]
            pend = []
            for sc, v in zip(scs, vs):
                sc = jnp.where(visible, sc * (scale * log2e), -1000000000.0 * log2e)
                e = jnp.exp2(sc - jnp.max(sc, axis=-1, keepdims=True))
                den = jnp.sum(e, axis=-1, keepdims=True)
                inv = pl.reciprocal(den, approx=True)
                pend.append((e, v, inv * (2.0 - den * inv)))
        best, best_idx = previous.finish()
        following.finish()
        outs = [None] * n_col
        order = CFG["wo_order"]
        if order == "g":
            order = [(g, j) for g in range(n_grp) for j in range(n_col)]
        elif order == "gj":
            order = [(g, j) for g in range(n_grp - 2) for j in range(n_col)] + [(g, j) for j in range(n_col) for g in range(n_grp - 2, n_grp)]
        for n, (g, j) in enumerate(order):
            if n == CFG["pv_last_at"] * n_col:
                heads[n_grp - 1] = attend(pend)
            w = pltpu.bitcast(wo[j, pl.ds(g * G * half, G * half), :], _BF16)
            t = _dot(heads[g], w)
            outs[j] = t if outs[j] is None else outs[j] + t
        out = jnp.concatenate(outs, axis=1)
        obuf[...] = out[M:]
        return out[:M], best, best_idx

    def out_copy(i):
        where = pl.ds(i * unroll, unroll)
        return pltpu.make_async_copy(xres.at[where], out_hbm.at[where], sems.at[5])

    def steps(i, carry, ahead):
        for u in range(unroll):
            carry = step(i * unroll + u, carry, u == 0, ahead)
        return carry

    def fresh():
        return (
            mem0_ref[...].astype(_F32),
            jnp.full((seg, 1), -np.inf, _F32),
            lax.broadcasted_iota(jnp.int32, (seg, 1), 0),
        )

    def layer(l, carry):
        def steps_and_store(i, carry):
            carry = steps(i, carry, False)

            @pl.when((l == 1) & (i > 0))
            def _():
                out_copy(i - 1).start()
            return carry

        _, best, best_idx = lax.fori_loop(
            jnp.where(l == 0, n_early // unroll, 0), n_seg // unroll, steps_and_store, carry)
        best, best_idx = _Staged(post(n_seg - 1, best, best_idx)).finish()

        @pl.when(l == 1)
        def _():
            out_copy(n_seg // unroll - 1).start()

        top = jnp.max(best, axis=0, keepdims=True)
        idx = jnp.min(jnp.where(best == top, best_idx, n_seg * seg - 1))

        x1 = x1buf[idx // seg]
        z1 = _layernorm(x1)
        gate = _rnd(_dot(z1, pltpu.bitcast(wg[...], _BF16)))
        g = _rnd(gate * _rnd(_sigmoid(gate)))
        u = _rnd(_dot(z1, pltpu.bitcast(wu[...], _BF16)))
        y = _rnd(_dot(g * u, pltpu.bitcast(wd[...], _BF16)))
        y = _rnd(y * _rnd(_sigmoid(top)))
        picked = lax.broadcasted_iota(jnp.int32, (seg, D), 0) == idx % seg
        x2 = (x1 + jnp.where(picked, _rnd(z1 + y), z1)).astype(_BF16)

        @pl.when(l == 0)
        def _():
            xres[idx // seg] = x2
            zbuf[0] = _layernorm(xres[0].astype(_F32))

        @pl.when(l == 1)
        def _():
            fixed[...] = x2
            for i in range(n_seg // unroll):
                out_copy(i).wait()
            fix_copy = pltpu.make_async_copy(fixed, out_hbm.at[idx // seg], sems.at[5])
            fix_copy.start()
            fix_copy.wait()

        return fresh()

    carry = lax.fori_loop(0, n_early // unroll, functools.partial(steps, ahead=True), fresh())
    for cp in [x_rest_copy] + ffn_copies:
        cp.wait()
    lax.fori_loop(0, 2, layer, carry)


@functools.partial(jax.jit, static_argnames=("A_seg_len",))
def pallas_interleave_layers__memory_aug_recurrent_mem_tr__moe_arch_mod__prompt_kernel(
    A_x: jax.Array,
    A_mem0: jax.Array,
    A_Wq: jax.Array,
    A_Wk: jax.Array,
    A_Wv: jax.Array,
    A_Wo: jax.Array,
    A_seg_len: int,
    B_x: jax.Array,
    B_w_r: jax.Array,
    B_w_gate: jax.Array,
    B_w_up: jax.Array,
    B_w_down: jax.Array,
):
    del B_x
    B, S, D = A_x.shape
    M = A_mem0.shape[1]
    H, Dh = A_Wq.shape[1:]
    F = B_w_gate.shape[1]
    seg = int(A_seg_len)
    n_seg = S // seg
    n_col = D // _LANES
    assert B == 1 and Dh == _LANES and S % seg == 0 and seg % 16 == 0 and M % 8 == 0
    early_rows = CFG["n_early"] * _EARLY

    hbm = pl.BlockSpec(memory_space=pl.ANY)
    vmem = pl.BlockSpec(memory_space=pltpu.VMEM)
    out = pl.pallas_call(
        functools.partial(_kernel, n_heads=H),
        out_shape=jax.ShapeDtypeStruct((n_seg, seg, D), A_x.dtype),
        in_specs=[hbm, vmem, hbm, hbm, hbm, hbm, vmem, hbm, hbm, hbm],
        out_specs=hbm,
        scratch_shapes=[
            pltpu.VMEM((3 * n_col, _LANES * H, Dh), _BF16),
            pltpu.VMEM((3, H, D // 2, Dh), _U32),
            pltpu.VMEM((n_col, H * Dh // 2, _LANES), _U32),
            pltpu.VMEM((D // 2, F), _U32),
            pltpu.VMEM((D // 2, F), _U32),
            pltpu.VMEM((F // 2, D), _U32),
            pltpu.VMEM((n_seg + 1, seg, D), _BF16),
            pltpu.VMEM((n_seg + 1, seg, D), _F32),
            pltpu.VMEM((n_seg + 1, seg, D), _F32),
            pltpu.VMEM((seg, D), _F32),
            pltpu.VMEM((n_col, early_rows, _LANES), _BF16 if CFG["zb"] else _F32),
            pltpu.VMEM((3, H, early_rows, Dh), _F32),
            pltpu.VMEM((seg, D), _BF16),
            pltpu.SemaphoreType.DMA((3 * n_col,)),
            pltpu.SemaphoreType.DMA((9,)),
        ],
        compiler_params=pltpu.CompilerParams(vmem_limit_bytes=100 * 1024 * 1024, flags=CFG["flags"]),
        name="rmt_mod",
    )(
        A_x.reshape(n_seg, seg, D),
        A_mem0.reshape(M, D),
        A_Wq.reshape(D * H, Dh),
        A_Wk.reshape(D * H, Dh),
        A_Wv.reshape(D * H, Dh),
        A_Wo.reshape(H * Dh, D),
        B_w_r.reshape(1, D),
        B_w_gate,
        B_w_up,
        B_w_down,
    )
    return out.reshape(B, S, D)
```

```python
import functools

import jax
import jax.numpy as jnp
import numpy as np
from jax import lax
import jax.experimental.pallas as pl
import jax.experimental.pallas.tpu as pltpu

CFG = dict(unroll=4, ksplit=1, wo_order="g", pv_last_at=3, G=4, post_pos=0, nshift=0, pack="kv", n_early=40, zb=1, flags=None, carry_z=0, xp=0, np=12, tp=1)


_F32 = jnp.float32
_BF16 = jnp.bfloat16
_U32 = jnp.uint32
_LANES = 128
_EARLY = 8
_NN = (((1,), (0,)), ((), ()))
_NT = (((1,), (1,)), ((), ()))
_K, _Q, _V = range(3)


def _dot(a, b, dims=_NN):
    return lax.dot_general(a, b, dims, preferred_element_type=_F32)


def _rnd(a):
    return a.astype(_BF16).astype(_F32)


def _layernorm_stages(x):
    inv_n = np.float32(1.0 / x.shape[-1])
    mean = jnp.sum(x, axis=-1, keepdims=True) * inv_n
    yield
    cen = x - mean
    var = jnp.sum(cen * cen, axis=-1, keepdims=True) * inv_n
    yield
    eps = np.float32(np.asarray(1e-05).astype(_BF16))
    den = _rnd(jnp.sqrt(_rnd(_rnd(var) + eps)))
    return _rnd(_rnd(x - _rnd(mean)) * (1.0 / den))


class _Staged:
    def __init__(self, stages):
        self._stages, self._result = stages, []

    def advance(self):
        if not self._result:
            try:
                next(self._stages)
            except StopIteration as done:
                self._result.append(done.value)

    def finish(self):
        while not self._result:
            self.advance()
        return self._result[0]


def _layernorm(x):
    return _Staged(_layernorm_stages(x)).finish()


def _sigmoid(x):
    return 1.0 / (1.0 + jnp.exp(-x))


def _kernel(
    x_hbm, mem0_ref, wq_hbm, wk_hbm, wv_hbm, wo_hbm, wr_ref, wg_hbm, wu_hbm, wd_hbm,
    out_hbm,
    wraw, wkqv, wo, wg, wu, wd, xres, zbuf, x1buf, obuf, zearly, early, fixed,
    w_sems, sems,
    *, n_heads,
):
    n_seg, seg, D = x_hbm.shape
    M = mem0_ref.shape[0]
    L = M + seg
    n_col = D // _LANES
    half = _LANES // 2
    scale = _LANES ** -0.5
    unroll = CFG["unroll"]
    n_early = CFG["n_early"]

    def x_copy(first, count, row, rows, sem):
        where = (pl.ds(first, count), pl.ds(row, rows))
        return pltpu.make_async_copy(x_hbm.at[where], xres.at[where], sems.at[sem])

    x_early_copy = x_copy(0, n_early, 0, _EARLY, 0)
    x_late_copy = x_copy(0, n_early, _EARLY, seg - _EARLY, 6)
    x_next_copy = x_copy(n_early, 1, 0, seg, 7)
    x_rest_copy = x_copy(n_early + 1, n_seg - n_early - 1, 0, seg, 8)
    wo_copies = [
        pltpu.make_async_copy(
            wo_hbm.at[:, pl.ds(j * _LANES, _LANES)], wo.at[j].bitcast(_BF16), sems.at[1])
        for j in range(n_col)
    ]
    ffn_copies = [
        pltpu.make_async_copy(src, dst.bitcast(_BF16), sems.at[2 + i])
        for i, (src, dst) in enumerate(((wg_hbm, wg), (wu_hbm, wu), (wd_hbm, wd)))
    ]
    x_early_copy.start(priority=CFG['xp'])
    for i, w in enumerate((wk_hbm, wq_hbm, wv_hbm)):
        for c in range(n_col):
            n = i * n_col + c
            pltpu.make_async_copy(
                w.at[pl.ds(c * _LANES * n_heads, _LANES * n_heads)], wraw.at[n], w_sems.at[n]
            ).start(priority=int(n < CFG['np']))

    xres[n_seg] = jnp.zeros((seg, D), _BF16)
    obuf[...] = jnp.zeros(obuf.shape, _F32)

    x_early_copy.wait()
    x = jnp.concatenate(
        [xres[t, pl.ds(0, _EARLY), :].astype(_F32) for t in range(n_early)], axis=0)
    z = _layernorm(x).astype(zearly.dtype)
    for c in range(n_col):
        zearly[c] = z[:, c * _LANES:(c + 1) * _LANES]

    def unpack_and_project(n, _):
        pltpu.make_async_copy(wraw.at[n], wraw.at[n], w_sems.at[n]).wait()

        @pl.when(n == n_col)
        def _():
            for cp in [x_late_copy, x_next_copy] + wo_copies:
                cp.start(priority=CFG['tp'])

        which, c = n // n_col, n % n_col
        words = wraw.at[n].bitcast(_U32)
        rows = pl.ds(pl.multiple_of(c * half, half), half)
        z = zearly[c]
        w_out, acc = wkqv.at[which], early.at[which]
        for p in range(n_heads // 2):
            w = words[pl.ds(p, _LANES, stride=n_heads // 2), :]
            pair = (w << 16, w & np.uint32(0xFFFF0000))
            for hd, bits in enumerate(pair, 2 * p):
                w_head = pltpu.bitcast(bits, _F32).astype(_BF16)
                w_out[hd, rows, :] = pltpu.bitcast(w_head, _U32)
                acc[hd] = _dot(z, w_head) + jnp.where(c > 0, acc[hd], 0.0)
    lax.fori_loop(0, 3 * n_col, unpack_and_project, None)

    for cp in [x_rest_copy] + ffn_copies:
        cp.start(priority=CFG['tp'])
    x_late_copy.wait()
    x_next_copy.wait()
    zbuf[0] = _layernorm(xres[0].astype(_F32))
    for cp in wo_copies:
        cp.wait()

    qi = lax.broadcasted_iota(jnp.int32, (L, L), 0)
    ki = lax.broadcasted_iota(jnp.int32, (L, L), 1)
    visible = (qi >= seg) | (ki >= seg) | (qi >= ki)
    w_r = wr_ref[...].astype(_F32)

    def post(s, best, best_idx):
        slot = jnp.where(s < 0, n_seg, s)
        x1 = _rnd(xres[slot].astype(_F32) + _rnd(obuf[...]))
        x1buf[slot] = x1
        z1 = yield from _layernorm_stages(x1)
        yield
        r = _rnd(jnp.sum(z1 * w_r, axis=-1, keepdims=True))
        idx = s * seg + lax.broadcasted_iota(jnp.int32, (seg, 1), 0)
        better = (r > best) & (idx >= 0)
        xres[slot] = (x1 + z1).astype(_BF16)
        return jnp.where(better, r, best), jnp.where(better, idx, best_idx)

    def pre(s):
        zbuf[s] = yield from _layernorm_stages(xres[s].astype(_F32))

    G = CFG["G"]
    n_grp = n_heads // G
    log2e = float(np.log2(np.e))

    def step(s, carry, first, ahead):
        mem, best, best_idx = carry
        heads = [None] * n_grp
        pend = None
        previous = _Staged(post(s - 1, best, best_idx))
        following = _Staged(pre(s + 1))
        if ahead:
            h = jnp.concatenate([zbuf[s, pl.ds(_EARLY, seg - _EARLY), :], mem], axis=0)
            early_rows = pl.ds(pl.multiple_of(s * _EARLY, _EARLY), _EARLY)
        else:
            h = jnp.concatenate([zbuf[s], mem], axis=0)

        def project(which, hds, by_column=False):
            if by_column:
                res = [None] * len(hds)
                for c in range(n_col):
                    for n, hd in enumerate(hds):
                        w = pltpu.bitcast(wkqv[which, hd, pl.ds(c * half, half), :], _BF16)
                        t = _dot(h[:, c * _LANES:(c + 1) * _LANES], w)
                        res[n] = t if c == 0 else res[n] + t
            else:
                res = [_dot(h, pltpu.bitcast(wkqv[which, hd], _BF16)) for hd in hds]
            if ahead:
                res = [jnp.concatenate([early[which, hd, early_rows, :], r], axis=0)
                       for hd, r in zip(hds, res)]
            if "kqv"[which] in CFG["pack"]:
                res = [r.astype(_BF16) for r in res]
            return res

        def attend(pend):
            o = jnp.concatenate([_dot(e, v) * inv for e, v, inv in pend], axis=1)
            return jnp.concatenate([o[seg:], o[:seg]], axis=0)

        for g in range(n_grp):
            if g >= CFG["post_pos"]:
                previous.advance()
            if g >= CFG["nshift"]:
                following.advance()
            hds = range(g * G, (g + 1) * G)
            ks = project(_K, hds, by_column=g == 0 and CFG["ksplit"] and not first)
            qs = project(_Q, hds)
            if pend is not None:
                heads[g - 1] = attend(pend)
            vs = project(_V, hds)
            scs = [_dot(q, k, _NT) for q, k in zip(qs, ks)]
            pend = []
            for sc, v in zip(scs, vs):
                sc = jnp.where(visible, sc * (scale * log2e), -1000000000.0 * log2e)
                e = jnp.exp2(sc - jnp.max(sc, axis=-1, keepdims=True))
                den = jnp.sum(e, axis=-1, keepdims=True)
                inv = pl.reciprocal(den, approx=True)
                pend.append((e, v, inv * (2.0 - den * inv)))
        best, best_idx = previous.finish()
        following.finish()
        outs = [None] * n_col
        order = CFG["wo_order"]
        if order == "g":
            order = [(g, j) for g in range(n_grp) for j in range(n_col)]
        elif order == "gj":
            order = [(g, j) for g in range(n_grp - 2) for j in range(n_col)] + [(g, j) for j in range(n_col) for g in range(n_grp - 2, n_grp)]
        for n, (g, j) in enumerate(order):
            if n == CFG["pv_last_at"] * n_col:
                heads[n_grp - 1] = attend(pend)
            w = pltpu.bitcast(wo[j, pl.ds(g * G * half, G * half), :], _BF16)
            t = _dot(heads[g], w)
            outs[j] = t if outs[j] is None else outs[j] + t
        out = jnp.concatenate(outs, axis=1)
        obuf[...] = out[M:]
        return out[:M], best, best_idx

    def out_copy(i):
        where = pl.ds(i * unroll, unroll)
        return pltpu.make_async_copy(xres.at[where], out_hbm.at[where], sems.at[5])

    def steps(i, carry, ahead):
        for u in range(unroll):
            carry = step(i * unroll + u, carry, u == 0, ahead)
        return carry

    def fresh():
        return (
            mem0_ref[...].astype(_F32),
            jnp.full((seg, 1), -np.inf, _F32),
            lax.broadcasted_iota(jnp.int32, (seg, 1), 0),
        )

    def layer(l, carry):
        def steps_and_store(i, carry):
            carry = steps(i, carry, False)

            @pl.when((l == 1) & (i > 0))
            def _():
                out_copy(i - 1).start()
            return carry

        _, best, best_idx = lax.fori_loop(
            jnp.where(l == 0, n_early // unroll, 0), n_seg // unroll, steps_and_store, carry)
        best, best_idx = _Staged(post(n_seg - 1, best, best_idx)).finish()

        @pl.when(l == 1)
        def _():
            out_copy(n_seg // unroll - 1).start()

        top = jnp.max(best, axis=0, keepdims=True)
        idx = jnp.min(jnp.where(best == top, best_idx, n_seg * seg - 1))

        x1 = x1buf[idx // seg]
        z1 = _layernorm(x1)
        gate = _rnd(_dot(z1, pltpu.bitcast(wg[...], _BF16)))
        g = _rnd(gate * _rnd(_sigmoid(gate)))
        u = _rnd(_dot(z1, pltpu.bitcast(wu[...], _BF16)))
        y = _rnd(_dot(g * u, pltpu.bitcast(wd[...], _BF16)))
        y = _rnd(y * _rnd(_sigmoid(top)))
        picked = lax.broadcasted_iota(jnp.int32, (seg, D), 0) == idx % seg
        x2 = (x1 + jnp.where(picked, _rnd(z1 + y), z1)).astype(_BF16)

        @pl.when(l == 0)
        def _():
            xres[idx // seg] = x2
            zbuf[0] = _layernorm(xres[0].astype(_F32))

        @pl.when(l == 1)
        def _():
            fixed[...] = x2
            for i in range(n_seg // unroll):
                out_copy(i).wait()
            fix_copy = pltpu.make_async_copy(fixed, out_hbm.at[idx // seg], sems.at[5])
            fix_copy.start()
            fix_copy.wait()

        return fresh()

    carry = lax.fori_loop(0, n_early // unroll, functools.partial(steps, ahead=True), fresh())
    for cp in [x_rest_copy] + ffn_copies:
        cp.wait()
    lax.fori_loop(0, 2, layer, carry)


@functools.partial(jax.jit, static_argnames=("A_seg_len",))
def pallas_interleave_layers__memory_aug_recurrent_mem_tr__moe_arch_mod__prompt_kernel(
    A_x: jax.Array,
    A_mem0: jax.Array,
    A_Wq: jax.Array,
    A_Wk: jax.Array,
    A_Wv: jax.Array,
    A_Wo: jax.Array,
    A_seg_len: int,
    B_x: jax.Array,
    B_w_r: jax.Array,
    B_w_gate: jax.Array,
    B_w_up: jax.Array,
    B_w_down: jax.Array,
):
    del B_x
    B, S, D = A_x.shape
    M = A_mem0.shape[1]
    H, Dh = A_Wq.shape[1:]
    F = B_w_gate.shape[1]
    seg = int(A_seg_len)
    n_seg = S // seg
    n_col = D // _LANES
    assert B == 1 and Dh == _LANES and S % seg == 0 and seg % 16 == 0 and M % 8 == 0
    early_rows = CFG["n_early"] * _EARLY

    hbm = pl.BlockSpec(memory_space=pl.ANY)
    vmem = pl.BlockSpec(memory_space=pltpu.VMEM)
    out = pl.pallas_call(
        functools.partial(_kernel, n_heads=H),
        out_shape=jax.ShapeDtypeStruct((n_seg, seg, D), A_x.dtype),
        in_specs=[hbm, vmem, hbm, hbm, hbm, hbm, vmem, hbm, hbm, hbm],
        out_specs=hbm,
        scratch_shapes=[
            pltpu.VMEM((3 * n_col, _LANES * H, Dh), _BF16),
            pltpu.VMEM((3, H, D // 2, Dh), _U32),
            pltpu.VMEM((n_col, H * Dh // 2, _LANES), _U32),
            pltpu.VMEM((D // 2, F), _U32),
            pltpu.VMEM((D // 2, F), _U32),
            pltpu.VMEM((F // 2, D), _U32),
            pltpu.VMEM((n_seg + 1, seg, D), _BF16),
            pltpu.VMEM((n_seg + 1, seg, D), _F32),
            pltpu.VMEM((n_seg + 1, seg, D), _F32),
            pltpu.VMEM((seg, D), _F32),
            pltpu.VMEM((n_col, early_rows, _LANES), _BF16 if CFG["zb"] else _F32),
            pltpu.VMEM((3, H, early_rows, Dh), _F32),
            pltpu.VMEM((seg, D), _BF16),
            pltpu.SemaphoreType.DMA((3 * n_col,)),
            pltpu.SemaphoreType.DMA((9,)),
        ],
        compiler_params=pltpu.CompilerParams(vmem_limit_bytes=100 * 1024 * 1024, flags=CFG["flags"]),
        name="rmt_mod",
    )(
        A_x.reshape(n_seg, seg, D),
        A_mem0.reshape(M, D),
        A_Wq.reshape(D * H, Dh),
        A_Wk.reshape(D * H, Dh),
        A_Wv.reshape(D * H, Dh),
        A_Wo.reshape(H * Dh, D),
        B_w_r.reshape(1, D),
        B_w_gate,
        B_w_up,
        B_w_down,
    )
    return out.reshape(B, S, D)
```

```python
import functools

import jax
import jax.numpy as jnp
import numpy as np
from jax import lax
import jax.experimental.pallas as pl
import jax.experimental.pallas.tpu as pltpu

_F32 = jnp.float32
_BF16 = jnp.bfloat16
_U32 = jnp.uint32
_LANES = 128
_HALF = _LANES // 2
_NN = (((1,), (0,)), ((), ()))
_NT = (((1,), (1,)), ((), ()))
_K, _Q, _V = range(3)

_GROUP = 4
_EARLY_ROWS = 8
_EARLY_SEGS = 40
_UNROLL_EARLY = 2
_UNROLL = 8


def _dot(a, b, dims=_NN):
    return lax.dot_general(a, b, dims, preferred_element_type=_F32)


def _rnd(a):
    return a.astype(_BF16).astype(_F32)


def _layernorm_stages(x):
    inv_n = np.float32(1.0 / x.shape[-1])
    mean = jnp.sum(x, axis=-1, keepdims=True) * inv_n
    yield
    cen = x - mean
    var = jnp.sum(cen * cen, axis=-1, keepdims=True) * inv_n
    yield
    eps = np.float32(np.asarray(1e-05).astype(_BF16))
    den = _rnd(jnp.sqrt(_rnd(_rnd(var) + eps)))
    return _rnd(_rnd(x - _rnd(mean)) * (1.0 / den))


class _Staged:
    def __init__(self, stages):
        self._stages, self._result = stages, []

    def advance(self):
        if not self._result:
            try:
                next(self._stages)
            except StopIteration as done:
                self._result.append(done.value)

    def finish(self):
        while not self._result:
            self.advance()
        return self._result[0]


def _layernorm(x):
    return _Staged(_layernorm_stages(x)).finish()


def _sigmoid(x):
    return 1.0 / (1.0 + jnp.exp(-x))


def _kernel(
    x_hbm, mem0_hbm, wq_hbm, wk_hbm, wv_hbm, wo_hbm, wr_hbm, wg_hbm, wu_hbm, wd_hbm,
    out_hbm,
    wraw, wkqv, wo, wg, wu, wd, mem0, wr,
    xres, zbuf, x1buf, z1buf, obuf, zearly, early, fixed,
    w_sems, in_sems, out_sem,
):
    n_seg, seg, D = x_hbm.shape
    n_heads = wkqv.shape[1]
    M = mem0.shape[0]
    L = M + seg
    n_col = D // _LANES
    n_grp = n_heads // _GROUP

    sem_ids = iter(range(in_sems.shape[0]))

    def copy(src, dst):
        return pltpu.make_async_copy(src, dst, in_sems.at[next(sem_ids)])

    def x_copy(first, count, row, rows):
        where = (pl.ds(first, count), pl.ds(row, rows))
        return copy(x_hbm.at[where], xres.at[where])

    late = seg - _EARLY_ROWS
    for_early = [x_copy(0, _EARLY_SEGS, 0, _EARLY_ROWS), x_copy(0, 1, _EARLY_ROWS, late)]
    for_steps = [
        x_copy(1, _EARLY_SEGS - 1, _EARLY_ROWS, late),
        x_copy(_EARLY_SEGS, 1, 0, seg),
        copy(mem0_hbm, mem0),
        copy(wr_hbm, wr),
    ] + [
        copy(wo_hbm.at[:, pl.ds(j * _LANES, _LANES)], wo.at[j].bitcast(_BF16))
        for j in range(n_col)
    ]
    for_later = [
        x_copy(_EARLY_SEGS + 1, n_seg - _EARLY_SEGS - 1, 0, seg),
        copy(wg_hbm, wg.bitcast(_BF16)),
        copy(wu_hbm, wu.bitcast(_BF16)),
        copy(wd_hbm, wd.bitcast(_BF16)),
    ]
    chunk = _LANES * n_heads

    for cp in for_early:
        cp.start()
    for which, w_hbm in ((_K, wk_hbm), (_Q, wq_hbm), (_V, wv_hbm)):
        for c in range(n_col):
            n = which * n_col + c
            pltpu.make_async_copy(
                w_hbm.at[pl.ds(c * chunk, chunk)], wraw.at[n, pl.ds(0, chunk)], w_sems.at[n]
            ).start(priority=1)

    xres[n_seg] = jnp.zeros((seg, D), _BF16)
    obuf[...] = jnp.zeros(obuf.shape, _F32)

    for cp in for_early:
        cp.wait()
    rows = [xres[t, pl.ds(0, _EARLY_ROWS), :].astype(_F32) for t in range(_EARLY_SEGS)]
    z = _layernorm(jnp.concatenate(rows, axis=0)).astype(_BF16)
    for c in range(n_col):
        zearly[c] = z[:, c * _LANES:(c + 1) * _LANES]
    zbuf[0] = _layernorm(xres[0].astype(_F32))

    def unpack_and_project(n, _):
        landed = wraw.at[n, pl.ds(0, chunk)]
        pltpu.make_async_copy(landed, landed, w_sems.at[n]).wait()
        which, c = n // n_col, n % n_col
        words = wraw.at[n].bitcast(_U32)
        depth = pl.ds(pl.multiple_of(c * _HALF, _HALF), _HALF)
        z = zearly[c]
        w_out, acc = wkqv.at[which], early.at[which]
        for p in range(n_heads // 2):
            w = words[pl.ds(p, _LANES, stride=n_heads // 2), :]
            for hd, bits in enumerate((w << 16, w & np.uint32(0xFFFF0000)), 2 * p):
                w_head = pltpu.bitcast(bits, _F32).astype(_BF16)
                w_out[hd, depth, :] = pltpu.bitcast(w_head, _U32)
                acc[hd] = _dot(z, w_head) + jnp.where(c > 0, acc[hd], 0.0)

    lax.fori_loop(0, n_col, unpack_and_project, None)
    for cp in for_steps:
        cp.start(priority=1)
    lax.fori_loop(n_col, 3 * n_col, unpack_and_project, None)
    for cp in for_steps:
        cp.wait()
    for cp in for_later:
        cp.start(priority=1)

    qi = lax.broadcasted_iota(jnp.int32, (L, L), 0)
    ki = lax.broadcasted_iota(jnp.int32, (L, L), 1)
    visible = (qi >= seg) | (ki >= seg) | (qi >= ki)
    log2e = float(np.log2(np.e))
    w_r = wr[...].astype(_F32).reshape(1, D)

    def before(s):
        zbuf[s] = yield from _layernorm_stages(xres[s].astype(_F32))

    def after(s, best, best_idx):
        slot = jnp.where(s < 0, n_seg, s)
        x1 = _rnd(xres[slot].astype(_F32) + _rnd(obuf[...]))
        x1buf[slot] = x1
        z1 = yield from _layernorm_stages(x1)
        z1buf[slot] = z1
        yield
        r = _rnd(jnp.sum(z1 * w_r, axis=-1, keepdims=True))
        idx = s * seg + lax.broadcasted_iota(jnp.int32, (seg, 1), 0)
        better = (r > best) & (idx >= 0)
        xres[slot] = (x1 + z1).astype(_BF16)
        return jnp.where(better, r, best), jnp.where(better, idx, best_idx)

    def softmax_parts(scores):
        scores = jnp.where(visible, scores * (_LANES ** -0.5 * log2e), -1000000000.0 * log2e)
        e = jnp.exp2(scores - jnp.max(scores, axis=-1, keepdims=True))
        den = jnp.sum(e, axis=-1, keepdims=True)
        inv = pl.reciprocal(den, approx=True)
        return e, inv * (2.0 - den * inv)

    def attend(pending):
        o = jnp.concatenate([_dot(e, v) * inv for (e, inv), v in pending], axis=1)
        return jnp.concatenate([o[seg:], o[:seg]], axis=0)

    def step(s, carry, mem_is_fresh, has_early):
        mem, best, best_idx = carry
        previous = _Staged(after(s - 1, best, best_idx))
        following = _Staged(before(s + 1))
        skip = _EARLY_ROWS if has_early else 0
        h = jnp.concatenate([zbuf[s, pl.ds(skip, seg - skip), :], mem], axis=0)

        def project(which, hds, by_column=False):
            if by_column:
                res = [None] * len(hds)
                for c in range(n_col):
                    for n, hd in enumerate(hds):
                        w = pltpu.bitcast(wkqv[which, hd, pl.ds(c * _HALF, _HALF), :], _BF16)
                        t = _dot(h[:, c * _LANES:(c + 1) * _LANES], w)
                        res[n] = t if c == 0 else res[n] + t
            else:
                res = [_dot(h, pltpu.bitcast(wkqv[which, hd], _BF16)) for hd in hds]
            if has_early:
                done = pl.ds(pl.multiple_of(s * skip, skip), skip)
                res = [jnp.concatenate([early[which, hd, done, :], r], axis=0)
                       for hd, r in zip(hds, res)]
            return res if which == _Q else [r.astype(_BF16) for r in res]

        heads, pending = [], None
        for g in range(n_grp):
            previous.advance()
            following.advance()
            hds = range(g * _GROUP, (g + 1) * _GROUP)
            ks = project(_K, hds, by_column=mem_is_fresh and g == 0)
            qs = project(_Q, hds)
            vs = project(_V, hds[:1])
            if pending:
                heads.append(attend(pending))
            vs += project(_V, hds[1:])
            scores = [_dot(q, k, _NT) for q, k in zip(qs, ks)]
            pending = [(softmax_parts(sc), v) for sc, v in zip(scores, vs)]
        best, best_idx = previous.finish()
        following.finish()

        outs = [None] * n_col
        for j0 in range(0, n_col, 2):
            for g in range(n_grp):
                if j0 == 0 and g == n_grp // 2:
                    heads.append(attend(pending))
                depth = pl.ds(g * _GROUP * _HALF, _GROUP * _HALF)
                for j in (j0, j0 + 1):
                    t = _dot(heads[g], pltpu.bitcast(wo[j, depth, :], _BF16))
                    outs[j] = t if g == 0 else outs[j] + t
        out = jnp.concatenate(outs, axis=1)
        obuf[...] = out[M:]
        return out[:M], best, best_idx

    def steps(i, carry, unroll, has_early):
        for u in range(unroll):
            carry = step(i * unroll + u, carry, u > 0, has_early)
        return carry

    def out_copy(i):
        where = pl.ds(i * _UNROLL, _UNROLL)
        return pltpu.make_async_copy(xres.at[where], out_hbm.at[where], out_sem)

    def layer_start():
        return (
            mem0[...].astype(_F32),
            jnp.full((seg, 1), -np.inf, _F32),
            lax.broadcasted_iota(jnp.int32, (seg, 1), 0),
        )

    def layer(l, carry):
        def steps_then_store(i, carry):
            carry = steps(i, carry, _UNROLL, False)

            @pl.when((l == 1) & (i > 0))
            def _():
                out_copy(i - 1).start()
            return carry

        first = jnp.where(l == 0, _EARLY_SEGS // _UNROLL, 0)
        _, best, best_idx = lax.fori_loop(first, n_seg // _UNROLL, steps_then_store, carry)
        best, best_idx = _Staged(after(n_seg - 1, best, best_idx)).finish()

        @pl.when(l == 1)
        def _():
            out_copy(n_seg // _UNROLL - 1).start()

        top = jnp.max(best, axis=0, keepdims=True)
        idx = jnp.min(jnp.where(best == top, best_idx, n_seg * seg - 1))

        zbuf[0] = _layernorm(xres[0].astype(_F32))
        z = z1buf[idx // seg, pl.ds(pl.multiple_of(idx % seg // 8 * 8, 8), 8), :]
        gate = _rnd(_dot(z, pltpu.bitcast(wg[...], _BF16)))
        g = _rnd(gate * _rnd(_sigmoid(gate)))
        u = _rnd(_dot(z, pltpu.bitcast(wu[...], _BF16)))
        y = _rnd(_dot(g * u, pltpu.bitcast(wd[...], _BF16)))
        y = _rnd(z + _rnd(y * _rnd(_sigmoid(top))))
        picked = lax.broadcasted_iota(jnp.int32, (seg, D), 0) == idx % seg
        z1 = jnp.where(picked, jnp.concatenate([y] * (seg // 8), axis=0), z1buf[idx // seg])
        x2 = (x1buf[idx // seg] + z1).astype(_BF16)

        @pl.when(l == 0)
        def _():
            xres[idx // seg] = x2

            @pl.when(idx < seg)
            def _():
                zbuf[0] = _layernorm(x2.astype(_F32))

        @pl.when(l == 1)
        def _():
            fixed[...] = x2
            for i in range(n_seg // _UNROLL):
                out_copy(i).wait()
            fix_copy = pltpu.make_async_copy(fixed, out_hbm.at[idx // seg], out_sem)
            fix_copy.start()
            fix_copy.wait()

        return layer_start()

    carry = lax.fori_loop(
        0, _EARLY_SEGS // _UNROLL_EARLY,
        functools.partial(steps, unroll=_UNROLL_EARLY, has_early=True), layer_start())
    for cp in for_later:
        cp.wait()
    lax.fori_loop(0, 2, layer, carry)


@functools.partial(jax.jit, static_argnames=("A_seg_len",))
def pallas_interleave_layers__memory_aug_recurrent_mem_tr__moe_arch_mod__prompt_kernel(
    A_x: jax.Array,
    A_mem0: jax.Array,
    A_Wq: jax.Array,
    A_Wk: jax.Array,
    A_Wv: jax.Array,
    A_Wo: jax.Array,
    A_seg_len: int,
    B_x: jax.Array,
    B_w_r: jax.Array,
    B_w_gate: jax.Array,
    B_w_up: jax.Array,
    B_w_down: jax.Array,
):
    del B_x
    B, S, D = A_x.shape
    M = A_mem0.shape[1]
    H, Dh = A_Wq.shape[1:]
    F = B_w_gate.shape[1]
    seg = int(A_seg_len)
    n_seg = S // seg
    n_col = D // _LANES
    assert B == 1 and Dh == _LANES and n_col % 2 == 0 and H % (2 * _GROUP) == 0
    assert S % seg == 0 and seg % 16 == 0 and M % 8 == 0
    assert n_seg % _UNROLL == 0 and n_seg > _EARLY_SEGS + 1
    n_early = _EARLY_SEGS * _EARLY_ROWS

    hbm = pl.BlockSpec(memory_space=pl.ANY)
    out = pl.pallas_call(
        _kernel,
        out_shape=jax.ShapeDtypeStruct((n_seg, seg, D), A_x.dtype),
        in_specs=[hbm] * 10,
        out_specs=hbm,
        scratch_shapes=[
            pltpu.VMEM((3 * n_col, (_LANES + 1) * H, Dh), _BF16),
            pltpu.VMEM((3, H, D // 2, Dh), _U32),
            pltpu.VMEM((n_col, H * Dh // 2, _LANES), _U32),
            pltpu.VMEM((D // 2, F), _U32),
            pltpu.VMEM((D // 2, F), _U32),
            pltpu.VMEM((F // 2, D), _U32),
            pltpu.VMEM((M, D), _BF16),
            pltpu.VMEM((D,), _BF16),
            pltpu.VMEM((n_seg + 1, seg, D), _BF16),
            pltpu.VMEM((n_seg + 1, seg, D), _F32),
            pltpu.VMEM((n_seg + 1, seg, D), _F32),
            pltpu.VMEM((n_seg + 1, seg, D), _F32),
            pltpu.VMEM((seg, D), _F32),
            pltpu.VMEM((n_col, n_early, _LANES), _BF16),
            pltpu.VMEM((3, H, n_early, Dh), _F32),
            pltpu.VMEM((seg, D), _BF16),
            pltpu.SemaphoreType.DMA((3 * n_col,)),
            pltpu.SemaphoreType.DMA((10 + n_col,)),
            pltpu.SemaphoreType.DMA,
        ],
        compiler_params=pltpu.CompilerParams(vmem_limit_bytes=100 * 1024 * 1024),
        name="rmt_mod",
    )(
        A_x.reshape(n_seg, seg, D),
        A_mem0.reshape(M, D),
        A_Wq.reshape(D * H, Dh),
        A_Wk.reshape(D * H, Dh),
        A_Wv.reshape(D * H, Dh),
        A_Wo.reshape(H * Dh, D),
        B_w_r,
        B_w_gate,
        B_w_up,
        B_w_down,
    )
    return out.reshape(B, S, D)
```

```python
import functools

import jax
import jax.numpy as jnp
import numpy as np
from jax import lax
import jax.experimental.pallas as pl
import jax.experimental.pallas.tpu as pltpu

_F32 = jnp.float32
_BF16 = jnp.bfloat16
_U32 = jnp.uint32
_LANES = 128
_HALF = _LANES // 2
_NN = (((1,), (0,)), ((), ()))
_NT = (((1,), (1,)), ((), ()))
_K, _Q, _V = range(3)

_GROUP = 4
_EARLY_ROWS = 8
_EARLY_SEGS = 40
_UNROLL_EARLY = 2
_UNROLL = 8


def _dot(a, b, dims=_NN):
    return lax.dot_general(a, b, dims, preferred_element_type=_F32)


def _rnd(a):
    return a.astype(_BF16).astype(_F32)


def _layernorm_stages(x):
    inv_n = np.float32(1.0 / x.shape[-1])
    mean = jnp.sum(x, axis=-1, keepdims=True) * inv_n
    yield
    cen = x - mean
    var = jnp.sum(cen * cen, axis=-1, keepdims=True) * inv_n
    yield
    eps = np.float32(np.asarray(1e-05).astype(_BF16))
    den = _rnd(jnp.sqrt(_rnd(_rnd(var) + eps)))
    return _rnd(_rnd(x - _rnd(mean)) * (1.0 / den))


class _Staged:
    def __init__(self, stages):
        self._stages, self._result = stages, []

    def advance(self):
        if not self._result:
            try:
                next(self._stages)
            except StopIteration as done:
                self._result.append(done.value)

    def finish(self):
        while not self._result:
            self.advance()
        return self._result[0]


def _layernorm(x):
    return _Staged(_layernorm_stages(x)).finish()


def _sigmoid(x):
    return 1.0 / (1.0 + jnp.exp(-x))


def _kernel(
    x_hbm, mem0_hbm, wq_hbm, wk_hbm, wv_hbm, wo_hbm, wr_hbm, wg_hbm, wu_hbm, wd_hbm,
    out_hbm,
    wraw, wkqv, wo, wg, wu, wd,
    xres, zbuf, x1buf, z1buf, obuf, zearly, early, fixed, mem0, wr,
    w_sems, in_sems, out_sem,
):
    n_seg, seg, D = x_hbm.shape
    n_heads = wkqv.shape[1]
    M = mem0.shape[0]
    L = M + seg
    n_col = D // _LANES
    n_grp = n_heads // _GROUP

    sem_ids = iter(range(in_sems.shape[0]))

    def copy(src, dst):
        return pltpu.make_async_copy(src, dst, in_sems.at[next(sem_ids)])

    def x_copy(first, count, row, rows):
        where = (pl.ds(first, count), pl.ds(row, rows))
        return copy(x_hbm.at[where], xres.at[where])

    late = seg - _EARLY_ROWS
    for_early = [x_copy(0, _EARLY_SEGS, 0, _EARLY_ROWS), x_copy(0, 1, _EARLY_ROWS, late)]
    for_steps = [
        x_copy(1, _EARLY_SEGS - 1, _EARLY_ROWS, late),
        x_copy(_EARLY_SEGS, 1, 0, seg),
        copy(mem0_hbm, mem0),
        copy(wr_hbm, wr),
    ] + [
        copy(wo_hbm.at[:, pl.ds(j * _LANES, _LANES)], wo.at[j].bitcast(_BF16))
        for j in range(n_col)
    ]
    for_later = [
        x_copy(_EARLY_SEGS + 1, n_seg - _EARLY_SEGS - 1, 0, seg),
        copy(wg_hbm, wg.bitcast(_BF16)),
        copy(wu_hbm, wu.bitcast(_BF16)),
        copy(wd_hbm, wd.bitcast(_BF16)),
    ]
    chunk = _LANES * n_heads

    def w_start(which, first, stop):
        def start(c, _):
            n = which * n_col + c
            src = (wk_hbm, wq_hbm, wv_hbm)[which]
            pltpu.make_async_copy(
                src.at[pl.ds(pl.multiple_of(c * chunk, chunk), chunk)],
                wraw.at[n, pl.ds(0, chunk)], w_sems.at[n]).start()
        lax.fori_loop(first, stop, start, None)

    for cp in for_early:
        cp.start()
    w_start(_K, 0, 1)

    xres[n_seg] = jnp.zeros((seg, D), _BF16)
    obuf[...] = jnp.zeros(obuf.shape, _F32)

    for cp in for_early:
        cp.wait()
    w_start(_K, 1, n_col)
    w_start(_Q, 0, n_col)
    w_start(_V, 0, n_col)
    for cp in for_steps:
        cp.start()
    rows = [xres[t, pl.ds(0, _EARLY_ROWS), :].astype(_F32) for t in range(_EARLY_SEGS)]
    z = _layernorm(jnp.concatenate(rows, axis=0)).astype(_BF16)
    for c in range(n_col):
        zearly[c] = z[:, c * _LANES:(c + 1) * _LANES]
    zbuf[0] = _layernorm(xres[0].astype(_F32))

    def unpack_and_project(n, _):
        landed = wraw.at[n, pl.ds(0, chunk)]
        pltpu.make_async_copy(landed, landed, w_sems.at[n]).wait()
        which, c = n // n_col, n % n_col
        words = wraw.at[n].bitcast(_U32)
        depth = pl.ds(pl.multiple_of(c * _HALF, _HALF), _HALF)
        z = zearly[c]
        w_out, acc = wkqv.at[which], early.at[which]
        for p in range(n_heads // 2):
            w = words[pl.ds(p, _LANES, stride=n_heads // 2), :]
            for hd, bits in enumerate((w << 16, w & np.uint32(0xFFFF0000)), 2 * p):
                w_head = pltpu.bitcast(bits, _F32).astype(_BF16)
                w_out[hd, depth, :] = pltpu.bitcast(w_head, _U32)
                acc[hd] = _dot(z, w_head) + jnp.where(c > 0, acc[hd], 0.0)

    lax.fori_loop(0, 3 * n_col, unpack_and_project, None)
    for cp in for_steps:
        cp.wait()
    for cp in for_later:
        cp.start()

    qi = lax.broadcasted_iota(jnp.int32, (L, L), 0)
    ki = lax.broadcasted_iota(jnp.int32, (L, L), 1)
    visible = (qi >= seg) | (ki >= seg) | (qi >= ki)
    log2e = float(np.log2(np.e))
    w_r = wr[...].astype(_F32).reshape(1, D)

    def before(s):
        zbuf[s] = yield from _layernorm_stages(xres[s].astype(_F32))

    def after(s, best, best_idx):
        slot = jnp.where(s < 0, n_seg, s)
        x1 = _rnd(xres[slot].astype(_F32) + _rnd(obuf[...]))
        x1buf[slot] = x1
        z1 = yield from _layernorm_stages(x1)
        z1buf[slot] = z1
        yield
        r = _rnd(jnp.sum(z1 * w_r, axis=-1, keepdims=True))
        idx = s * seg + lax.broadcasted_iota(jnp.int32, (seg, 1), 0)
        better = (r > best) & (idx >= 0)
        xres[slot] = (x1 + z1).astype(_BF16)
        return jnp.where(better, r, best), jnp.where(better, idx, best_idx)

    def softmax_parts(scores):
        scores = jnp.where(visible, scores * (_LANES ** -0.5 * log2e), -1000000000.0 * log2e)
        e = jnp.exp2(scores - jnp.max(scores, axis=-1, keepdims=True))
        den = jnp.sum(e, axis=-1, keepdims=True)
        inv = pl.reciprocal(den, approx=True)
        return e, inv * (2.0 - den * inv)

    def attend(pending):
        o = jnp.concatenate([_dot(e, v) * inv for (e, inv), v in pending], axis=1)
        return jnp.concatenate([o[seg:], o[:seg]], axis=0)

    def step(s, carry, mem_is_fresh, has_early):
        mem, best, best_idx = carry
        previous = _Staged(after(s - 1, best, best_idx))
        following = _Staged(before(s + 1))
        skip = _EARLY_ROWS if has_early else 0
        h = jnp.concatenate([zbuf[s, pl.ds(skip, seg - skip), :], mem], axis=0)

        def project(which, hds, by_column=False):
            if by_column:
                res = [None] * len(hds)
                for c in range(n_col):
                    for n, hd in enumerate(hds):
                        w = pltpu.bitcast(wkqv[which, hd, pl.ds(c * _HALF, _HALF), :], _BF16)
                        t = _dot(h[:, c * _LANES:(c + 1) * _LANES], w)
                        res[n] = t if c == 0 else res[n] + t
            else:
                res = [_dot(h, pltpu.bitcast(wkqv[which, hd], _BF16)) for hd in hds]
            if has_early:
                done = pl.ds(pl.multiple_of(s * skip, skip), skip)
                res = [jnp.concatenate([early[which, hd, done, :], r], axis=0)
                       for hd, r in zip(hds, res)]
            return res if which == _Q else [r.astype(_BF16) for r in res]

        heads, pending = [], None
        for g in range(n_grp):
            previous.advance()
            following.advance()
            hds = range(g * _GROUP, (g + 1) * _GROUP)
            ks = project(_K, hds, by_column=mem_is_fresh and g == 0)
            qs = project(_Q, hds)
            vs = project(_V, hds[:1])
            if pending:
                heads.append(attend(pending))
            vs += project(_V, hds[1:])
            scores = [_dot(q, k, _NT) for q, k in zip(qs, ks)]
            pending = [(softmax_parts(sc), v) for sc, v in zip(scores, vs)]
        best, best_idx = previous.finish()
        following.finish()

        outs = [None] * n_col
        for j0 in range(0, n_col, 2):
            for g in range(n_grp):
                if j0 == 0 and g == n_grp // 2:
                    heads.append(attend(pending))
                depth = pl.ds(g * _GROUP * _HALF, _GROUP * _HALF)
                for j in (j0, j0 + 1):
                    t = _dot(heads[g], pltpu.bitcast(wo[j, depth, :], _BF16))
                    outs[j] = t if g == 0 else outs[j] + t
        out = jnp.concatenate(outs, axis=1)
        obuf[...] = out[M:]
        return out[:M], best, best_idx

    def steps(i, carry, unroll, has_early):
        for u in range(unroll):
            carry = step(i * unroll + u, carry, u > 0, has_early)
        return carry

    def out_copy(i):
        where = pl.ds(i * _UNROLL, _UNROLL)
        return pltpu.make_async_copy(xres.at[where], out_hbm.at[where], out_sem)

    def layer_start():
        return (
            mem0[...].astype(_F32),
            jnp.full((seg, 1), -np.inf, _F32),
            lax.broadcasted_iota(jnp.int32, (seg, 1), 0),
        )

    def layer(l, carry):
        def steps_then_store(i, carry):
            carry = steps(i, carry, _UNROLL, False)

            @pl.when((l == 1) & (i > 0))
            def _():
                out_copy(i - 1).start()
            return carry

        first = jnp.where(l == 0, _EARLY_SEGS // _UNROLL, 0)
        _, best, best_idx = lax.fori_loop(first, n_seg // _UNROLL, steps_then_store, carry)
        best, best_idx = _Staged(after(n_seg - 1, best, best_idx)).finish()

        @pl.when(l == 1)
        def _():
            out_copy(n_seg // _UNROLL - 1).start()

        top = jnp.max(best, axis=0, keepdims=True)
        idx = jnp.min(jnp.where(best == top, best_idx, n_seg * seg - 1))

        zbuf[0] = _layernorm(xres[0].astype(_F32))
        z = z1buf[idx // seg, pl.ds(pl.multiple_of(idx % seg // 8 * 8, 8), 8), :]
        gate = _rnd(_dot(z, pltpu.bitcast(wg[...], _BF16)))
        g = _rnd(gate * _rnd(_sigmoid(gate)))
        u = _rnd(_dot(z, pltpu.bitcast(wu[...], _BF16)))
        y = _rnd(_dot(g * u, pltpu.bitcast(wd[...], _BF16)))
        y = _rnd(z + _rnd(y * _rnd(_sigmoid(top))))
        picked = lax.broadcasted_iota(jnp.int32, (seg, D), 0) == idx % seg
        z1 = jnp.where(picked, jnp.concatenate([y] * (seg // 8), axis=0), z1buf[idx // seg])
        x2 = (x1buf[idx // seg] + z1).astype(_BF16)

        @pl.when(l == 0)
        def _():
            xres[idx // seg] = x2

            @pl.when(idx < seg)
            def _():
                zbuf[0] = _layernorm(x2.astype(_F32))

        @pl.when(l == 1)
        def _():
            fixed[...] = x2
            for i in range(n_seg // _UNROLL):
                out_copy(i).wait()
            fix_copy = pltpu.make_async_copy(fixed, out_hbm.at[idx // seg], out_sem)
            fix_copy.start()
            fix_copy.wait()

        return layer_start()

    carry = lax.fori_loop(
        0, _EARLY_SEGS // _UNROLL_EARLY,
        functools.partial(steps, unroll=_UNROLL_EARLY, has_early=True), layer_start())
    for cp in for_later:
        cp.wait()
    lax.fori_loop(0, 2, layer, carry)


@functools.partial(jax.jit, static_argnames=("A_seg_len",))
def pallas_interleave_layers__memory_aug_recurrent_mem_tr__moe_arch_mod__prompt_kernel(
    A_x: jax.Array,
    A_mem0: jax.Array,
    A_Wq: jax.Array,
    A_Wk: jax.Array,
    A_Wv: jax.Array,
    A_Wo: jax.Array,
    A_seg_len: int,
    B_x: jax.Array,
    B_w_r: jax.Array,
    B_w_gate: jax.Array,
    B_w_up: jax.Array,
    B_w_down: jax.Array,
):
    del B_x
    B, S, D = A_x.shape
    M = A_mem0.shape[1]
    H, Dh = A_Wq.shape[1:]
    F = B_w_gate.shape[1]
    seg = int(A_seg_len)
    n_seg = S // seg
    n_col = D // _LANES
    assert B == 1 and Dh == _LANES and n_col % 2 == 0 and H % (2 * _GROUP) == 0
    assert S % seg == 0 and seg % 16 == 0 and M % 8 == 0
    assert n_seg % _UNROLL == 0 and n_seg > _EARLY_SEGS + 1
    n_early = _EARLY_SEGS * _EARLY_ROWS

    hbm = pl.BlockSpec(memory_space=pl.ANY)
    out = pl.pallas_call(
        _kernel,
        out_shape=jax.ShapeDtypeStruct((n_seg, seg, D), A_x.dtype),
        in_specs=[hbm] * 10,
        out_specs=hbm,
        scratch_shapes=[
            pltpu.VMEM((3 * n_col, (_LANES + 1) * H, Dh), _BF16),
            pltpu.VMEM((3, H, D // 2, Dh), _U32),
            pltpu.VMEM((n_col, H * Dh // 2, _LANES), _U32),
            pltpu.VMEM((D // 2, F), _U32),
            pltpu.VMEM((D // 2, F), _U32),
            pltpu.VMEM((F // 2, D), _U32),
            pltpu.VMEM((n_seg + 1, seg, D), _BF16),
            pltpu.VMEM((n_seg + 1, seg, D), _F32),
            pltpu.VMEM((n_seg + 1, seg, D), _F32),
            pltpu.VMEM((n_seg + 1, seg, D), _F32),
            pltpu.VMEM((seg, D), _F32),
            pltpu.VMEM((n_col, n_early, _LANES), _BF16),
            pltpu.VMEM((3, H, n_early, Dh), _F32),
            pltpu.VMEM((seg, D), _BF16),
            pltpu.VMEM((M, D), _BF16),
            pltpu.VMEM((D,), _BF16),
            pltpu.SemaphoreType.DMA((3 * n_col,)),
            pltpu.SemaphoreType.DMA((10 + n_col,)),
            pltpu.SemaphoreType.DMA,
        ],
        compiler_params=pltpu.CompilerParams(vmem_limit_bytes=100 * 1024 * 1024),
        name="rmt_mod",
    )(
        A_x.reshape(n_seg, seg, D),
        A_mem0.reshape(M, D),
        A_Wq.reshape(D * H, Dh),
        A_Wk.reshape(D * H, Dh),
        A_Wv.reshape(D * H, Dh),
        A_Wo.reshape(H * Dh, D),
        B_w_r,
        B_w_gate,
        B_w_up,
        B_w_down,
    )
    return out.reshape(B, S, D)
```

```python
import functools

import jax
import jax.numpy as jnp
import numpy as np
from jax import lax
import jax.experimental.pallas as pl
import jax.experimental.pallas.tpu as pltpu

_F32 = jnp.float32
_BF16 = jnp.bfloat16
_U32 = jnp.uint32
_LANES = 128
_HALF = _LANES // 2
_NN = (((1,), (0,)), ((), ()))
_NT = (((1,), (1,)), ((), ()))
_K, _Q, _V = range(3)

_GROUP = 4
_EARLY_ROWS = 8
_EARLY_SEGS = 40
_UNROLL_EARLY = 2
_UNROLL = 8


def _dot(a, b, dims=_NN):
    return lax.dot_general(a, b, dims, preferred_element_type=_F32)


def _rnd(a):
    return a.astype(_BF16).astype(_F32)


def _layernorm_stages(x):
    inv_n = np.float32(1.0 / x.shape[-1])
    mean = jnp.sum(x, axis=-1, keepdims=True) * inv_n
    yield
    cen = x - mean
    var = jnp.sum(cen * cen, axis=-1, keepdims=True) * inv_n
    yield
    eps = np.float32(np.asarray(1e-05).astype(_BF16))
    den = _rnd(jnp.sqrt(_rnd(_rnd(var) + eps)))
    return _rnd(_rnd(x - _rnd(mean)) * (1.0 / den))


class _Staged:
    def __init__(self, stages):
        self._stages, self._result = stages, []

    def advance(self):
        if not self._result:
            try:
                next(self._stages)
            except StopIteration as done:
                self._result.append(done.value)

    def finish(self):
        while not self._result:
            self.advance()
        return self._result[0]


def _layernorm(x):
    return _Staged(_layernorm_stages(x)).finish()


def _sigmoid(x):
    return 1.0 / (1.0 + jnp.exp(-x))


def _kernel(
    x_hbm, mem0_hbm, wq_hbm, wk_hbm, wv_hbm, wo_hbm, wr_hbm, wg_hbm, wu_hbm, wd_hbm,
    out_hbm,
    wraw, wkqv, wo, wg, wu, wd,
    xres, zbuf, x1buf, z1buf, obuf, zearly, early, fixed, mem0, wr,
    w_sems, in_sems, out_sem,
):
    n_seg, seg, D = x_hbm.shape
    n_heads = wkqv.shape[1]
    M = mem0.shape[0]
    L = M + seg
    n_col = D // _LANES
    n_grp = n_heads // _GROUP

    sem_ids = iter(range(in_sems.shape[0]))

    def copy(src, dst):
        return pltpu.make_async_copy(src, dst, in_sems.at[next(sem_ids)])

    def x_copy(first, count, row, rows):
        where = (pl.ds(first, count), pl.ds(row, rows))
        return copy(x_hbm.at[where], xres.at[where])

    late = seg - _EARLY_ROWS
    for_early = [x_copy(0, _EARLY_SEGS, 0, _EARLY_ROWS), x_copy(0, 1, _EARLY_ROWS, late)]
    for_steps = [
        x_copy(1, _EARLY_SEGS - 1, _EARLY_ROWS, late),
        x_copy(_EARLY_SEGS, 1, 0, seg),
        copy(mem0_hbm, mem0),
        copy(wr_hbm, wr),
    ] + [
        copy(wo_hbm.at[:, pl.ds(j * _LANES, _LANES)], wo.at[j])
        for j in range(n_col)
    ]
    for_later = [
        x_copy(_EARLY_SEGS + 1, n_seg - _EARLY_SEGS - 1, 0, seg),
        copy(wg_hbm, wg),
        copy(wu_hbm, wu),
        copy(wd_hbm, wd),
    ]
    chunk = _LANES * n_heads

    def w_start(which, first, stop):
        def start(c, _):
            n = which * n_col + c
            src = (wk_hbm, wq_hbm, wv_hbm)[which]
            pltpu.make_async_copy(
                src.at[pl.ds(pl.multiple_of(c * chunk, chunk), chunk)],
                wraw.at[n, pl.ds(0, chunk)], w_sems.at[n]).start()
        lax.fori_loop(first, stop, start, None)

    for cp in for_early:
        cp.start()
    w_start(_K, 0, 1)

    xres[n_seg] = jnp.zeros((seg, D), _BF16)
    obuf[...] = jnp.zeros(obuf.shape, _F32)

    for cp in for_early:
        cp.wait()
    w_start(_K, 1, n_col)
    w_start(_Q, 0, n_col)
    w_start(_V, 0, n_col)
    for cp in for_steps:
        cp.start()
    rows = [xres[t, pl.ds(0, _EARLY_ROWS), :].astype(_F32) for t in range(_EARLY_SEGS)]
    z = _layernorm(jnp.concatenate(rows, axis=0)).astype(_BF16)
    for c in range(n_col):
        zearly[c] = z[:, c * _LANES:(c + 1) * _LANES]
    zbuf[0] = _layernorm(xres[0].astype(_F32))

    def unpack_and_project(n, _):
        landed = wraw.at[n, pl.ds(0, chunk)]
        pltpu.make_async_copy(landed, landed, w_sems.at[n]).wait()
        which, c = n // n_col, n % n_col
        words = wraw.at[n].bitcast(_U32)
        depth = pl.ds(pl.multiple_of(c * _HALF, _HALF), _HALF)
        z = zearly[c]
        w_out, acc = wkqv.at[which], early.at[which]
        for p in range(n_heads // 2):
            w = words[pl.ds(p, _LANES, stride=n_heads // 2), :]
            for hd, bits in enumerate((w << 16, w & np.uint32(0xFFFF0000)), 2 * p):
                w_head = pltpu.bitcast(bits, _F32).astype(_BF16)
                w_out[hd, depth, :] = pltpu.bitcast(w_head, _U32)
                acc[hd] = _dot(z, w_head) + jnp.where(c > 0, acc[hd], 0.0)

    lax.fori_loop(0, 3 * n_col, unpack_and_project, None)
    for cp in for_steps:
        cp.wait()
    for cp in for_later:
        cp.start()

    qi = lax.broadcasted_iota(jnp.int32, (L, L), 0)
    ki = lax.broadcasted_iota(jnp.int32, (L, L), 1)
    visible = (qi >= seg) | (ki >= seg) | (qi >= ki)
    log2e = float(np.log2(np.e))
    w_r = wr[...].astype(_F32).reshape(1, D)

    def before(s):
        zbuf[s] = yield from _layernorm_stages(xres[s].astype(_F32))

    def after(s, best, best_idx):
        slot = jnp.where(s < 0, n_seg, s)
        x1 = _rnd(xres[slot].astype(_F32) + _rnd(obuf[...]))
        x1buf[slot] = x1
        z1 = yield from _layernorm_stages(x1)
        z1buf[slot] = z1
        yield
        r = _rnd(jnp.sum(z1 * w_r, axis=-1, keepdims=True))
        idx = s * seg + lax.broadcasted_iota(jnp.int32, (seg, 1), 0)
        better = (r > best) & (idx >= 0)
        xres[slot] = (x1 + z1).astype(_BF16)
        return jnp.where(better, r, best), jnp.where(better, idx, best_idx)

    def softmax_parts(scores):
        scores = jnp.where(visible, scores * (_LANES ** -0.5 * log2e), -1000000000.0 * log2e)
        e = jnp.exp2(scores - jnp.max(scores, axis=-1, keepdims=True))
        den = jnp.sum(e, axis=-1, keepdims=True)
        inv = pl.reciprocal(den, approx=True)
        return e, inv * (2.0 - den * inv)

    def attend(pending):
        o = jnp.concatenate([_dot(e, v) * inv for (e, inv), v in pending], axis=1)
        return jnp.concatenate([o[seg:], o[:seg]], axis=0)

    def step(s, carry, mem_is_fresh, has_early):
        mem, best, best_idx = carry
        previous = _Staged(after(s - 1, best, best_idx))
        following = _Staged(before(s + 1))
        skip = _EARLY_ROWS if has_early else 0
        h = jnp.concatenate([zbuf[s, pl.ds(skip, seg - skip), :], mem], axis=0)

        def project(which, hds, by_column=False):
            if by_column:
                res = [None] * len(hds)
                for c in range(n_col):
                    for n, hd in enumerate(hds):
                        w = pltpu.bitcast(wkqv[which, hd, pl.ds(c * _HALF, _HALF), :], _BF16)
                        t = _dot(h[:, c * _LANES:(c + 1) * _LANES], w)
                        res[n] = t if c == 0 else res[n] + t
            else:
                res = [_dot(h, pltpu.bitcast(wkqv[which, hd], _BF16)) for hd in hds]
            if has_early:
                done = pl.ds(pl.multiple_of(s * skip, skip), skip)
                res = [jnp.concatenate([early[which, hd, done, :], r], axis=0)
                       for hd, r in zip(hds, res)]
            return res if which == _Q else [r.astype(_BF16) for r in res]

        heads, pending = [], None
        for g in range(n_grp):
            previous.advance()
            following.advance()
            hds = range(g * _GROUP, (g + 1) * _GROUP)
            ks = project(_K, hds, by_column=mem_is_fresh and g == 0)
            qs = project(_Q, hds)
            vs = project(_V, hds[:1])
            if pending:
                heads.append(attend(pending))
            vs += project(_V, hds[1:])
            scores = [_dot(q, k, _NT) for q, k in zip(qs, ks)]
            pending = [(softmax_parts(sc), v) for sc, v in zip(scores, vs)]
        best, best_idx = previous.finish()
        following.finish()

        outs = [None] * n_col
        for j0 in range(0, n_col, 2):
            for g in range(n_grp):
                if j0 == 0 and g == n_grp // 2:
                    heads.append(attend(pending))
                depth = pl.ds(g * _GROUP * _HALF, _GROUP * _HALF)
                for j in (j0, j0 + 1):
                    t = _dot(heads[g], pltpu.bitcast(wo.bitcast(_U32)[j, depth, :], _BF16))
                    outs[j] = t if g == 0 else outs[j] + t
        out = jnp.concatenate(outs, axis=1)
        obuf[...] = out[M:]
        return out[:M], best, best_idx

    def steps(i, carry, unroll, has_early):
        for u in range(unroll):
            carry = step(i * unroll + u, carry, u > 0, has_early)
        return carry

    def out_copy(i):
        where = pl.ds(i * _UNROLL, _UNROLL)
        return pltpu.make_async_copy(xres.at[where], out_hbm.at[where], out_sem)

    def layer_start():
        return (
            mem0[...].astype(_F32),
            jnp.full((seg, 1), -np.inf, _F32),
            lax.broadcasted_iota(jnp.int32, (seg, 1), 0),
        )

    def layer(l, carry):
        def steps_then_store(i, carry):
            carry = steps(i, carry, _UNROLL, False)

            @pl.when((l == 1) & (i > 0))
            def _():
                out_copy(i - 1).start()
            return carry

        first = jnp.where(l == 0, _EARLY_SEGS // _UNROLL, 0)
        _, best, best_idx = lax.fori_loop(first, n_seg // _UNROLL, steps_then_store, carry)
        best, best_idx = _Staged(after(n_seg - 1, best, best_idx)).finish()

        @pl.when(l == 1)
        def _():
            out_copy(n_seg // _UNROLL - 1).start()

        top = jnp.max(best, axis=0, keepdims=True)
        idx = jnp.min(jnp.where(best == top, best_idx, n_seg * seg - 1))

        zbuf[0] = _layernorm(xres[0].astype(_F32))
        z = z1buf[idx // seg, pl.ds(pl.multiple_of(idx % seg // 8 * 8, 8), 8), :]
        gate = _rnd(_dot(z, wg[...]))
        g = _rnd(gate * _rnd(_sigmoid(gate)))
        u = _rnd(_dot(z, wu[...]))
        y = _rnd(_dot(g * u, wd[...]))
        y = _rnd(z + _rnd(y * _rnd(_sigmoid(top))))
        picked = lax.broadcasted_iota(jnp.int32, (seg, D), 0) == idx % seg
        z1 = jnp.where(picked, jnp.concatenate([y] * (seg // 8), axis=0), z1buf[idx // seg])
        x2 = (x1buf[idx // seg] + z1).astype(_BF16)

        @pl.when(l == 0)
        def _():
            xres[idx // seg] = x2

            @pl.when(idx < seg)
            def _():
                zbuf[0] = _layernorm(x2.astype(_F32))

        @pl.when(l == 1)
        def _():
            fixed[...] = x2
            for i in range(n_seg // _UNROLL):
                out_copy(i).wait()
            fix_copy = pltpu.make_async_copy(fixed, out_hbm.at[idx // seg], out_sem)
            fix_copy.start()
            fix_copy.wait()

        return layer_start()

    carry = lax.fori_loop(
        0, _EARLY_SEGS // _UNROLL_EARLY,
        functools.partial(steps, unroll=_UNROLL_EARLY, has_early=True), layer_start())
    for cp in for_later:
        cp.wait()
    lax.fori_loop(0, 2, layer, carry)


@functools.partial(jax.jit, static_argnames=("A_seg_len",))
def pallas_interleave_layers__memory_aug_recurrent_mem_tr__moe_arch_mod__prompt_kernel(
    A_x: jax.Array,
    A_mem0: jax.Array,
    A_Wq: jax.Array,
    A_Wk: jax.Array,
    A_Wv: jax.Array,
    A_Wo: jax.Array,
    A_seg_len: int,
    B_x: jax.Array,
    B_w_r: jax.Array,
    B_w_gate: jax.Array,
    B_w_up: jax.Array,
    B_w_down: jax.Array,
):
    del B_x
    B, S, D = A_x.shape
    M = A_mem0.shape[1]
    H, Dh = A_Wq.shape[1:]
    F = B_w_gate.shape[1]
    seg = int(A_seg_len)
    n_seg = S // seg
    n_col = D // _LANES
    assert B == 1 and Dh == _LANES and n_col % 2 == 0 and H % (2 * _GROUP) == 0
    assert S % seg == 0 and seg % 16 == 0 and M % 8 == 0
    assert n_seg % _UNROLL == 0 and n_seg > _EARLY_SEGS + 1
    n_early = _EARLY_SEGS * _EARLY_ROWS

    hbm = pl.BlockSpec(memory_space=pl.ANY)
    out = pl.pallas_call(
        _kernel,
        out_shape=jax.ShapeDtypeStruct((n_seg, seg, D), A_x.dtype),
        in_specs=[hbm] * 10,
        out_specs=hbm,
        scratch_shapes=[
            pltpu.VMEM((3 * n_col, (_LANES + 1) * H, Dh), _BF16),
            pltpu.VMEM((3, H, D // 2, Dh), _U32),
            pltpu.VMEM((n_col, H * Dh, _LANES), _BF16),
            pltpu.VMEM((D, F), _BF16),
            pltpu.VMEM((D, F), _BF16),
            pltpu.VMEM((F, D), _BF16),
            pltpu.VMEM((n_seg + 1, seg, D), _BF16),
            pltpu.VMEM((n_seg + 1, seg, D), _F32),
            pltpu.VMEM((n_seg + 1, seg, D), _F32),
            pltpu.VMEM((n_seg + 1, seg, D), _F32),
            pltpu.VMEM((seg, D), _F32),
            pltpu.VMEM((n_col, n_early, _LANES), _BF16),
            pltpu.VMEM((3, H, n_early, Dh), _F32),
            pltpu.VMEM((seg, D), _BF16),
            pltpu.VMEM((M, D), _BF16),
            pltpu.VMEM((D,), _BF16),
            pltpu.SemaphoreType.DMA((3 * n_col,)),
            pltpu.SemaphoreType.DMA((10 + n_col,)),
            pltpu.SemaphoreType.DMA,
        ],
        compiler_params=pltpu.CompilerParams(vmem_limit_bytes=100 * 1024 * 1024),
        name="rmt_mod",
    )(
        A_x.reshape(n_seg, seg, D),
        A_mem0.reshape(M, D),
        A_Wq.reshape(D * H, Dh),
        A_Wk.reshape(D * H, Dh),
        A_Wv.reshape(D * H, Dh),
        A_Wo.reshape(H * Dh, D),
        B_w_r,
        B_w_gate,
        B_w_up,
        B_w_down,
    )
    return out.reshape(B, S, D)
```

```python
import functools

import jax
import jax.numpy as jnp
import numpy as np
from jax import lax
import jax.experimental.pallas as pl
import jax.experimental.pallas.tpu as pltpu

_F32 = jnp.float32
_BF16 = jnp.bfloat16
_U32 = jnp.uint32
_LANES = 128
_HALF = _LANES // 2
_NN = (((1,), (0,)), ((), ()))
_NT = (((1,), (1,)), ((), ()))
_K, _Q, _V = range(3)
_reciprocal = pltpu.reciprocal if hasattr(pltpu, "reciprocal") else pl.reciprocal

_GROUP = 4
_EARLY_ROWS = 8
_EARLY_SEGS = 40
_UNROLL_EARLY = 2
_UNROLL = 8


def _dot(a, b, dims=_NN):
    return lax.dot_general(a, b, dims, preferred_element_type=_F32)


def _rnd(a):
    return a.astype(_BF16).astype(_F32)


def _layernorm_stages(x):
    inv_n = np.float32(1.0 / x.shape[-1])
    mean = jnp.sum(x, axis=-1, keepdims=True) * inv_n
    yield
    cen = x - mean
    var = jnp.sum(cen * cen, axis=-1, keepdims=True) * inv_n
    yield
    eps = np.float32(np.asarray(1e-05).astype(_BF16))
    den = _rnd(jnp.sqrt(_rnd(_rnd(var) + eps)))
    return _rnd(_rnd(x - _rnd(mean)) * (1.0 / den))


class _Staged:
    def __init__(self, stages):
        self._stages, self._result = stages, []

    def advance(self):
        if not self._result:
            try:
                next(self._stages)
            except StopIteration as done:
                self._result.append(done.value)

    def finish(self):
        while not self._result:
            self.advance()
        return self._result[0]


def _layernorm(x):
    return _Staged(_layernorm_stages(x)).finish()


def _sigmoid(x):
    return 1.0 / (1.0 + jnp.exp(-x))


def _kernel(
    x_hbm, mem0_hbm, wq_hbm, wk_hbm, wv_hbm, wo_hbm, wr_hbm, wg_hbm, wu_hbm, wd_hbm,
    out_hbm,
    wraw, wkqv, wo, wg, wu, wd,
    xres, zbuf, x1buf, z1buf, obuf, zearly, early, fixed, mem0, wr,
    w_sems, in_sems, out_sem,
):
    n_seg, seg, D = x_hbm.shape
    n_heads = wkqv.shape[1]
    M = mem0.shape[0]
    L = M + seg
    n_col = D // _LANES
    n_grp = n_heads // _GROUP

    sem_ids = iter(range(in_sems.shape[0]))

    def copy(src, dst):
        return pltpu.make_async_copy(src, dst, in_sems.at[next(sem_ids)])

    def x_copy(first, count, row, rows):
        where = (pl.ds(first, count), pl.ds(row, rows))
        return copy(x_hbm.at[where], xres.at[where])

    late = seg - _EARLY_ROWS
    for_early = [x_copy(0, _EARLY_SEGS, 0, _EARLY_ROWS), x_copy(0, 1, _EARLY_ROWS, late)]
    for_steps = [
        x_copy(1, _EARLY_SEGS - 1, _EARLY_ROWS, late),
        x_copy(_EARLY_SEGS, 1, 0, seg),
        copy(mem0_hbm, mem0),
        copy(wr_hbm, wr),
    ] + [
        copy(wo_hbm.at[:, pl.ds(j * _LANES, _LANES)], wo.at[j])
        for j in range(n_col)
    ]
    for_later = [
        x_copy(_EARLY_SEGS + 1, n_seg - _EARLY_SEGS - 1, 0, seg),
        copy(wg_hbm, wg),
        copy(wu_hbm, wu),
        copy(wd_hbm, wd),
    ]
    chunk = _LANES * n_heads

    def w_start(which, first, stop):
        def start(c, _):
            n = which * n_col + c
            src = (wk_hbm, wq_hbm, wv_hbm)[which]
            pltpu.make_async_copy(
                src.at[pl.ds(pl.multiple_of(c * chunk, chunk), chunk)],
                wraw.at[n, pl.ds(0, chunk)], w_sems.at[n]).start()
        lax.fori_loop(first, stop, start, None)

    for cp in for_early:
        cp.start()
    w_start(_K, 0, 1)

    xres[n_seg] = jnp.zeros((seg, D), _BF16)
    obuf[...] = jnp.zeros(obuf.shape, _F32)

    for cp in for_early:
        cp.wait()
    w_start(_K, 1, n_col)
    w_start(_Q, 0, n_col)
    w_start(_V, 0, n_col)
    rows = [xres[t, pl.ds(0, _EARLY_ROWS), :].astype(_F32) for t in range(_EARLY_SEGS)]
    z = _layernorm(jnp.concatenate(rows, axis=0)).astype(_BF16)
    for c in range(n_col):
        zearly[c] = z[:, c * _LANES:(c + 1) * _LANES]
    zbuf[0] = _layernorm(xres[0].astype(_F32))
    for cp in for_steps:
        cp.start()

    def unpack_and_project(n, _):
        landed = wraw.at[n, pl.ds(0, chunk)]
        pltpu.make_async_copy(landed, landed, w_sems.at[n]).wait()
        which, c = n // n_col, n % n_col
        words = wraw.at[n].bitcast(_U32)
        depth = pl.ds(pl.multiple_of(c * _HALF, _HALF), _HALF)
        z = zearly[c]
        w_out, acc = wkqv.at[which], early.at[which]
        for p in range(n_heads // 2):
            w = words[pl.ds(p, _LANES, stride=n_heads // 2), :]
            for hd, bits in enumerate((w << 16, w & np.uint32(0xFFFF0000)), 2 * p):
                w_head = pltpu.bitcast(bits, _F32).astype(_BF16)
                w_out[hd, depth, :] = pltpu.bitcast(w_head, _U32)
                acc[hd] = _dot(z, w_head) + jnp.where(c > 0, acc[hd], 0.0)

    lax.fori_loop(0, 3 * n_col, unpack_and_project, None)
    for cp in for_steps:
        cp.wait()
    for cp in for_later:
        cp.start()

    qi = lax.broadcasted_iota(jnp.int32, (L, _LANES), 0)
    lane = lax.broadcasted_iota(jnp.int32, (L, _LANES), 1)
    ki = lane - jnp.where(lane >= 2 * L, 2 * L, jnp.where(lane >= L, L, 0))
    visible = (qi >= seg) | (ki >= seg) | (qi >= ki)
    log2e = float(np.log2(np.e))
    w_r = wr[...].astype(_F32).reshape(1, D)

    def before(s):
        zbuf[s] = yield from _layernorm_stages(xres[s].astype(_F32))

    def after(s, best, best_idx):
        slot = jnp.where(s < 0, n_seg, s)
        x1 = _rnd(xres[slot].astype(_F32) + _rnd(obuf[...]))
        x1buf[slot] = x1
        z1 = yield from _layernorm_stages(x1)
        z1buf[slot] = z1
        yield
        r = _rnd(jnp.sum(z1 * w_r, axis=-1, keepdims=True))
        idx = s * seg + lax.broadcasted_iota(jnp.int32, (seg, 1), 0)
        better = (r > best) & (idx >= 0)
        xres[slot] = (x1 + z1).astype(_BF16)
        return jnp.where(better, r, best), jnp.where(better, idx, best_idx)

    def window(i, rows=L):
        lane = lax.broadcasted_iota(jnp.int32, (rows, _LANES), 1)
        return (lane >= i * L) & (lane < (i + 1) * L)

    def merge(parts):
        out = parts[-1]
        for i in reversed(range(len(parts) - 1)):
            out = jnp.where(window(i), parts[i], out)
        return out

    def tile(parts):
        rest = _LANES - sum(p.shape[0] for p in parts)
        return jnp.concatenate(parts + ([jnp.zeros((rest, _LANES), _F32)] if rest else []), axis=0)

    def logits(scores):
        seen = visible[:, :scores.shape[1]]
        return jnp.where(seen, scores * (_LANES ** -0.5 * log2e), -1000000000.0 * log2e)

    def inverse(den):
        inv = _reciprocal(den, approx=True)
        return inv * (2.0 - den * inv)

    def softmax_windows(scores, n):
        scores = logits(scores)
        across = lambda per_window: merge([jnp.broadcast_to(t, scores.shape) for t in per_window])
        top = across([jnp.max(jnp.where(window(i), scores, -np.inf), axis=-1, keepdims=True)
                      for i in range(n)])
        e = jnp.exp2(jnp.where(lane < n * L, scores - top, -np.inf))
        den = across([jnp.sum(jnp.where(window(i), e, 0.0), axis=-1, keepdims=True)
                      for i in range(n)])
        return e * inverse(den)

    def attend_by_trio(project, advance, put):
        n_stage = n_heads // 6
        spare = range(6 * n_stage, n_heads)
        zero = jnp.zeros((L, _LANES), _F32)
        k, q, v = have = {}, {}, {}

        def need(which, hds, **kw):
            hds = [hd for hd in hds if hd not in have[which]]
            have[which].update(zip(hds, project(which, hds, **kw)))

        def trios(t):
            return [range(6 * t, 6 * t + 3), range(6 * t + 3, 6 * t + 6)]

        def inside(xs, hds):
            return tile([jnp.where(window(i), xs[hd], 0.0) for i, hd in enumerate(hds)]).astype(_BF16)

        def outside(i, k_t, q_head, p, v_head):
            k_t = jnp.where(window(i, _LANES), k_t, 0.0)
            rows = [k_t[:i * L]] if i else []
            rows += [jnp.where(window(i), 0.0, v_head), k_t[(i + 1) * L:]]
            return _dot(jnp.where(window(i), p, q_head), tile(rows).astype(_BF16))

        advance()
        first = list(range(6)) + list(spare)
        need(_K, first[:_GROUP], first=True)
        need(_K, first)
        need(_Q, first)
        need(_K, (6, 7))
        sets = trios(0) + [spare]
        scores = [merge([_dot(q[hd], tile([zero] * i + [k[hd]]).astype(_BF16), _NT)
                         for i, hd in enumerate(hds)]) for hds in sets]
        *probs, spare_prob = [softmax_windows(sc, len(hds)) for sc, hds in zip(scores, sets)]
        for t in range(1, n_stage):
            advance()
            need(_K, range(6 * t, 6 * t + 6))
            need(_V, range(6 * t - 6, 6 * t))
            need(_Q, range(6 * t, 6 * t + 6))
            if t + 1 < n_stage:
                need(_K, (6 * t + 6, 6 * t + 7))
            else:
                need(_V, spare)
            k_ts = [tile([k[hd] for hd in new]).T for new in trios(t)]
            o_in = [_dot(p, inside(v, old)) for p, old in zip(probs, trios(t - 1))]
            mixed, s_in = [], []
            for k_t, p, new, old in zip(k_ts, probs, trios(t), trios(t - 1)):
                mixed.append([outside(i, k_t, q[new[i]], p, v[old[i]]) for i in range(3)])
                s_in.append(_dot(merge([q[hd] for hd in new]), inside(k, new), _NT))
            for o, xs, old in zip(o_in, mixed, trios(t - 1)):
                put(old, [jnp.where(window(i), o, x) for i, x in enumerate(xs)])
            probs = [softmax_windows(merge(xs) + sc, 3) for xs, sc in zip(mixed, s_in)]
        need(_V, range(n_heads))

        def last():
            for p, hds in zip([spare_prob] + probs, [spare] + trios(n_stage - 1)):
                put(hds, [
                    _dot(p[:, :(i + 1) * L],
                         jnp.concatenate([zero] * i + [v[hd]], axis=0).astype(_BF16))
                    for i, hd in enumerate(hds)])
        return last

    def attend_by_head(project, advance, put):
        packed = lambda xs: [x.astype(_BF16) for x in xs]
        pending = None
        for g in range(n_grp):
            advance()
            hds = range(g * _GROUP, (g + 1) * _GROUP)
            ks = packed(project(_K, hds, first=g == 0))
            qs = project(_Q, hds)
            vs = packed(project(_V, hds[:1]))
            if pending:
                pending()
            vs += packed(project(_V, hds[1:]))
            parts = []
            for sc in [_dot(q, k, _NT) for q, k in zip(qs, ks)]:
                sc = logits(sc)
                e = jnp.exp2(sc - jnp.max(sc, axis=-1, keepdims=True))
                parts.append((e, inverse(jnp.sum(e, axis=-1, keepdims=True))))

            def pending(hds=hds, parts=parts, vs=vs):
                os = [_dot(e, v) for (e, _), v in zip(parts, vs)]
                put(hds, [o * inv for o, (_, inv) in zip(os, parts)])
        return pending

    def step(s, carry, mem_is_fresh, has_early):
        mem, best, best_idx = carry
        previous = _Staged(after(s - 1, best, best_idx))
        following = _Staged(before(s + 1))
        skip = _EARLY_ROWS if has_early else 0
        h = jnp.concatenate([zbuf[s, pl.ds(skip, seg - skip), :], mem], axis=0)

        def project(which, hds, first=False):
            if first and mem_is_fresh:
                res = [None] * len(hds)
                for c in range(n_col):
                    for n, hd in enumerate(hds):
                        w = pltpu.bitcast(wkqv[which, hd, pl.ds(c * _HALF, _HALF), :], _BF16)
                        t = _dot(h[:, c * _LANES:(c + 1) * _LANES], w)
                        res[n] = t if c == 0 else res[n] + t
            else:
                res = [_dot(h, pltpu.bitcast(wkqv[which, hd], _BF16)) for hd in hds]
            if has_early:
                done = pl.ds(pl.multiple_of(s * skip, skip), skip)
                res = [jnp.concatenate([early[which, hd, done, :], r], axis=0)
                       for hd, r in zip(hds, res)]
            return res

        def advance():
            previous.advance()
            following.advance()

        heads = [None] * n_heads

        def put(hds, os):
            for hd, o in zip(hds, os):
                heads[hd] = jnp.concatenate([o[seg:], o[:seg]], axis=0)

        last = (attend_by_head if has_early else attend_by_trio)(project, advance, put)
        best, best_idx = previous.finish()
        following.finish()

        outs = [None] * n_col
        for j0 in range(0, n_col, 2):
            for g in range(n_grp):
                if j0 == 0 and g == n_grp // 2:
                    last()
                depth = pl.ds(g * _GROUP * _HALF, _GROUP * _HALF)
                o = jnp.concatenate(heads[g * _GROUP:(g + 1) * _GROUP], axis=1)
                for j in (j0, j0 + 1):
                    t = _dot(o, pltpu.bitcast(wo.bitcast(_U32)[j, depth, :], _BF16))
                    outs[j] = t if g == 0 else outs[j] + t
        out = jnp.concatenate(outs, axis=1)
        obuf[...] = out[M:]
        return out[:M], best, best_idx

    def steps(i, carry, unroll, has_early):
        for u in range(unroll):
            carry = step(i * unroll + u, carry, u > 0, has_early)
        return carry

    def out_copy(i):
        where = pl.ds(i * _UNROLL, _UNROLL)
        return pltpu.make_async_copy(xres.at[where], out_hbm.at[where], out_sem)

    def layer_start():
        return (
            mem0[...].astype(_F32),
            jnp.full((seg, 1), -np.inf, _F32),
            lax.broadcasted_iota(jnp.int32, (seg, 1), 0),
        )

    def layer(l, carry):
        def steps_then_store(i, carry):
            carry = steps(i, carry, _UNROLL, False)

            @pl.when((l == 1) & (i > 0))
            def _():
                out_copy(i - 1).start()
            return carry

        first = jnp.where(l == 0, _EARLY_SEGS // _UNROLL, 0)
        _, best, best_idx = lax.fori_loop(first, n_seg // _UNROLL, steps_then_store, carry)
        best, best_idx = _Staged(after(n_seg - 1, best, best_idx)).finish()

        @pl.when(l == 1)
        def _():
            out_copy(n_seg // _UNROLL - 1).start()

        top = jnp.max(best, axis=0, keepdims=True)
        idx = jnp.min(jnp.where(best == top, best_idx, n_seg * seg - 1))

        zbuf[0] = _layernorm(xres[0].astype(_F32))
        z = z1buf[idx // seg, pl.ds(pl.multiple_of(idx % seg // 8 * 8, 8), 8), :]
        gate = _rnd(_dot(z, wg[...]))
        g = _rnd(gate * _rnd(_sigmoid(gate)))
        u = _rnd(_dot(z, wu[...]))
        y = _rnd(_dot(g * u, wd[...]))
        y = _rnd(z + _rnd(y * _rnd(_sigmoid(top))))
        picked = lax.broadcasted_iota(jnp.int32, (seg, D), 0) == idx % seg
        z1 = jnp.where(picked, jnp.concatenate([y] * (seg // 8), axis=0), z1buf[idx // seg])
        x2 = (x1buf[idx // seg] + z1).astype(_BF16)

        @pl.when(l == 0)
        def _():
            xres[idx // seg] = x2

            @pl.when(idx < seg)
            def _():
                zbuf[0] = _layernorm(x2.astype(_F32))

        @pl.when(l == 1)
        def _():
            fixed[...] = x2
            for i in range(n_seg // _UNROLL):
                out_copy(i).wait()
            fix_copy = pltpu.make_async_copy(fixed, out_hbm.at[idx // seg], out_sem)
            fix_copy.start()
            fix_copy.wait()

        return layer_start()

    carry = lax.fori_loop(
        0, _EARLY_SEGS // _UNROLL_EARLY,
        functools.partial(steps, unroll=_UNROLL_EARLY, has_early=True), layer_start())
    for cp in for_later:
        cp.wait()
    lax.fori_loop(0, 2, layer, carry)


@functools.partial(jax.jit, static_argnames=("A_seg_len",))
def pallas_interleave_layers__memory_aug_recurrent_mem_tr__moe_arch_mod__prompt_kernel(
    A_x: jax.Array,
    A_mem0: jax.Array,
    A_Wq: jax.Array,
    A_Wk: jax.Array,
    A_Wv: jax.Array,
    A_Wo: jax.Array,
    A_seg_len: int,
    B_x: jax.Array,
    B_w_r: jax.Array,
    B_w_gate: jax.Array,
    B_w_up: jax.Array,
    B_w_down: jax.Array,
):
    del B_x
    B, S, D = A_x.shape
    M = A_mem0.shape[1]
    H, Dh = A_Wq.shape[1:]
    F = B_w_gate.shape[1]
    seg = int(A_seg_len)
    n_seg = S // seg
    n_col = D // _LANES
    assert B == 1 and Dh == _LANES and n_col % 2 == 0 and H % _GROUP == 0 and H % 6 == 2
    assert S % seg == 0 and seg % 16 == 0 and M % 8 == 0 and 3 * (M + seg) <= _LANES
    assert n_seg % _UNROLL == 0 and n_seg > _EARLY_SEGS + 1
    n_early = _EARLY_SEGS * _EARLY_ROWS

    hbm = pl.BlockSpec(memory_space=pl.ANY)
    out = pl.pallas_call(
        _kernel,
        out_shape=jax.ShapeDtypeStruct((n_seg, seg, D), A_x.dtype),
        in_specs=[hbm] * 10,
        out_specs=hbm,
        scratch_shapes=[
            pltpu.VMEM((3 * n_col, (_LANES + 1) * H, Dh), _BF16),
            pltpu.VMEM((3, H, D // 2, Dh), _U32),
            pltpu.VMEM((n_col, H * Dh, _LANES), _BF16),
            pltpu.VMEM((D, F), _BF16),
            pltpu.VMEM((D, F), _BF16),
            pltpu.VMEM((F, D), _BF16),
            pltpu.VMEM((n_seg + 1, seg, D), _BF16),
            pltpu.VMEM((n_seg + 1, seg, D), _F32),
            pltpu.VMEM((n_seg + 1, seg, D), _F32),
            pltpu.VMEM((n_seg + 1, seg, D), _F32),
            pltpu.VMEM((seg, D), _F32),
            pltpu.VMEM((n_col, n_early, _LANES), _BF16),
            pltpu.VMEM((3, H, n_early, Dh), _F32),
            pltpu.VMEM((seg, D), _BF16),
            pltpu.VMEM((M, D), _BF16),
            pltpu.VMEM((D,), _BF16),
            pltpu.SemaphoreType.DMA((3 * n_col,)),
            pltpu.SemaphoreType.DMA((10 + n_col,)),
            pltpu.SemaphoreType.DMA,
        ],
        compiler_params=pltpu.CompilerParams(vmem_limit_bytes=100 * 1024 * 1024),
        name="rmt_mod",
    )(
        A_x.reshape(n_seg, seg, D),
        A_mem0.reshape(M, D),
        A_Wq.reshape(D * H, Dh),
        A_Wk.reshape(D * H, Dh),
        A_Wv.reshape(D * H, Dh),
        A_Wo.reshape(H * Dh, D),
        B_w_r,
        B_w_gate,
        B_w_up,
        B_w_down,
    )
    return out.reshape(B, S, D)
```
